```python
import os as _os
_os.environ.setdefault("JAX_PLATFORMS", "cpu")
import jax
import jax.numpy as jnp

def _softmax(x, axis=-1):
    return jax.nn.softmax(x, axis=axis)
def _gelu(x):
    return jax.nn.gelu(x, approximate=True)
def _silu(x):
    return jax.nn.silu(x)
def _sigmoid(x):
    return jax.nn.sigmoid(x)
def _layernorm(x, axis=-1, eps=1e-5):
    m = jnp.mean(x, axis=axis, keepdims=True)
    v = jnp.var(x, axis=axis, keepdims=True)
    return (x - m) / jnp.sqrt(v + eps)
def _scatter_add(tgt, idx, src, axis=0):
    return tgt.at[idx].add(src)
def _segment_sum(src, seg, n):
    return jax.ops.segment_sum(src, seg, n)
class _Rng:
    def __init__(self, key):
        self._k = key
    def _next(self):
        self._k, sub = jax.random.split(self._k)
        return sub
    def normal(self, shape):
        return jax.random.normal(self._next(), shape, dtype=jnp.bfloat16)
    def randint(self, lo, hi, shape):
        return jax.random.randint(self._next(), shape, lo, hi, dtype=jnp.int32)
    def uniform(self, shape, lo=0.0, hi=1.0):
        return jax.random.uniform(self._next(), shape, jnp.bfloat16, lo, hi)
    def permutation(self, n):
        return jax.random.permutation(self._next(), n)


kernel_name = 'sequential_preLN__softmax_full_mha__dense_activation_gelu__prompt'

def setup_inputs():
    _rng = _Rng(jax.random.key(int.from_bytes(__import__("os").urandom(4), "little")))
    _w = (lambda a: (lambda t: t.astype(jnp.bfloat16) if jnp.issubdtype(t.dtype, jnp.floating) else t)(jnp.asarray(a)))
    def _A_setup():
        B, S, D = 1, 2048, 512
        return {
            "x": _w((lambda *s: _rng.normal(s) * 0.05)(B, S, D)),
            "wqkv": _w((lambda *s: _rng.normal(s) * 0.05)(D, 3 * D)),
            "wo": _w((lambda *s: _rng.normal(s) * 0.05)(D, D)),
        }
    _A_in = _A_setup()

    def _B_setup():
        B, S, D, F = 1, 2048, 512, 1792
        return {
            "x": _w((lambda *s: _rng.normal(s) * 0.05)(B, S, D)),
            "w1": _w((lambda *s: _rng.normal(s) * 0.4)(D, F) * (D ** -0.5)),
            "b1": _w((lambda *s: _rng.normal(s) * 0.4)(F) * 0.01),
            "w2": _w((lambda *s: _rng.normal(s) * 0.4)(F, D) * (F ** -0.5)),
            "b2": _w((lambda *s: _rng.normal(s) * 0.05)(D) * 0.01),
        }
    _B_in = _B_setup()

    return {
        "A_x": _A_in["x"],
        "A_wqkv": _A_in["wqkv"],
        "A_wo": _A_in["wo"],
        "B_x": _B_in["x"],
        "B_w1": _B_in["w1"],
        "B_b1": _B_in["b1"],
        "B_w2": _B_in["w2"],
        "B_b2": _B_in["b2"],
    }

def reference(A_x, A_wqkv, A_wo, B_x, B_w1, B_b1, B_w2, B_b2):
    def _A_ref(x, wqkv, wo):
        B, S, D = x.shape
        H = 32; Dh = D // H
        qkv = (lambda x, *d: x.transpose(*d))((x @ wqkv).reshape(B, S, 3, H, Dh), 2, 0, 3, 1, 4)
        q, k, v = qkv[0], qkv[1], qkv[2]
        scale = Dh ** -0.5
        scores = jnp.einsum("bhqd,bhkd->bhqk", q, k) * scale
        p = _softmax(scores, axis=-1)
        o = jnp.einsum("bhqk,bhkd->bhqd", p, v)
        return (lambda x, *d: x.transpose(*d))(o, 0, 2, 1, 3).reshape(B, S, D) @ wo

    def _B_ref(x, w1, b1, w2, b2):
        h = jnp.einsum("bsd,df->bsf", x, w1) + b1
        h = _gelu(h)
        return jnp.einsum("bsf,fd->bsd", h, w2) + b2

    x = A_x
    h = x + _A_ref(_layernorm(x, axis=-1), A_wqkv, A_wo)
    h2 = h + _B_ref(_layernorm(h, axis=-1), B_w1, B_b1, B_w2, B_b2)
    return h2
```

```python
import math, contextlib
import jax, jax.numpy as jnp
from jax import lax
from jax.experimental import pallas as pl
from jax.experimental.pallas import tpu as pltpu

S, D, H, DH, F = 2048, 512, 32, 16, 1792
LOG2E = 1.4426950408889634
f32, bf16, u32 = jnp.float32, jnp.bfloat16, jnp.uint32

def _ln(x):
    m = jnp.mean(x, axis=-1, keepdims=True)
    xc = x - m
    v = jnp.mean(xc * xc, axis=-1, keepdims=True)
    return xc * lax.rsqrt(v + 1e-5)

def _gelu(x):
    c = math.sqrt(2.0 / math.pi)
    return 0.5 * x * (1.0 + jnp.tanh(c * (x + 0.044715 * (x * x * x))))

NT = (((1,), (1,)), ((), ()))

def _make(lag=10, vpos=0, off=9, share=2, nacc=1, scopes=0, force_fb=0, taper=40, fb=1):
    TQ = 512
    PC = 512
    TK = 128
    NQ = S // TQ
    NK = S // TK
    NL = TQ // 128
    GM = 7
    HU = 8
    NZ = HU * NK * 8 // share
    TS = 256
    L_LO, L_HI = 2.0 ** -20, 2.0 ** 60
    scope = (lambda n: jax.named_scope(n)) if scopes else (lambda n: contextlib.nullcontext())
    def kernel(x_hbm, wqkv_hbm, wo_hbm, w1_hbm, b1_hbm, w2_hbm, b2_hbm, o_ref,
               x_scr, xv_scr, wq_scr, wk_scr, wv_scr, wo_scr, w1_scr, w2_scr, sems,
               k_scr, kb_scr, qt_scr, qf_scr, vt_scr, ot_scr, zacc, z_ref, zs_ref, bad_scr, b1_scr, b2_scr):
        i = pl.program_id(0)
        CPC = PC // TK
        cp_xv = pltpu.make_async_copy(x_hbm.at[:, vpos * 16:vpos * 16 + 16, :], xv_scr, sems.at[0])
        cp_wk = pltpu.make_async_copy(wqkv_hbm.at[:, D:2 * D], wk_scr, sems.at[1])
        cp_wq = pltpu.make_async_copy(wqkv_hbm.at[:, 0:D], wq_scr, sems.at[2])
        cp_wv = pltpu.make_async_copy(wqkv_hbm.at[:, 2 * D:3 * D], wv_scr, sems.at[3])
        cp_x = [pltpu.make_async_copy(x_hbm.at[c * CPC:(c + 1) * CPC], x_scr.at[c], sems.at[4 + c]) for c in range(4)]
        cp_late = [pltpu.make_async_copy(wo_hbm, wo_scr, sems.at[8]),
                   pltpu.make_async_copy(w1_hbm, w1_scr, sems.at[9]),
                   pltpu.make_async_copy(b1_hbm, b1_scr, sems.at[10]),
                   pltpu.make_async_copy(w2_hbm, w2_scr, sems.at[11]),
                   pltpu.make_async_copy(b2_hbm, b2_scr, sems.at[12])]

        def _prologue():
            cp_xv.start()
            cp_wk.start()
            cp_x[0].start()
            cp_wq.start()
            cp_wv.start()
            for c in range(1, 4):
                cp_x[c].start()
            zacc[...] = jnp.zeros_like(zacc)
            z_ref[...] = jnp.zeros_like(z_ref)
            for n in range(NZ):
                zs_ref[n] = 0
            cp_xv.wait()
            xv = xv_scr[...].reshape(NK * 16, D).astype(f32)
            lnv = _ln(xv).astype(bf16)
            cp_wk.wait()
            wk = wk_scr[...]
            kv = pltpu.bitcast(jnp.dot(lnv, wk, preferred_element_type=f32).astype(bf16), u32)
            for s in range(4):
                for j in range(NK):
                    k_scr[s, (j * 8 + vpos) * 8:(j * 8 + vpos) * 8 + 8, :] = kv[j * 8:(j + 1) * 8, s * 128:(s + 1) * 128]
            lanes = iter(range(128))
            def kb_some(n):
                for _ in range(n):
                    c = next(lanes)
                    for s in range(4):
                        b = jnp.broadcast_to(kv[:, s * 128 + c:s * 128 + c + 1], (128, 128))
                        kb_scr[s, c] = pltpu.bitcast(b, bf16).astype(f32)
            wqT = wvT = vmax = None
            for c in range(S // PC):
                cp_x[c].wait()
                if c == 1:
                    for cp in cp_late:
                        cp.start()
                x = x_scr[c].reshape(PC, D).astype(f32)
                ln = _ln(x).astype(bf16)
                rows = []
                for jj in range(CPC):
                    if vpos > 0:
                        rows.append(ln[jj * TK:jj * TK + vpos * 16])
                    if vpos < 7:
                        rows.append(ln[jj * TK + vpos * 16 + 16:(jj + 1) * TK])
                lnm = jnp.concatenate(rows, axis=0)
                if c == 0:
                    cp_wq.wait()
                    wqT = wq_scr[...].astype(f32).T.astype(bf16)
                kb_some(10)
                k = pltpu.bitcast(jnp.dot(lnm, wk, preferred_element_type=f32).astype(bf16), u32)
                for s in range(4):
                    for jj in range(CPC):
                        j = c * CPC + jj
                        if vpos > 0:
                            k_scr[s, j * 64:j * 64 + vpos * 8, :] = k[jj * 56:jj * 56 + vpos * 8, s * 128:(s + 1) * 128]
                        if vpos < 7:
                            k_scr[s, j * 64 + vpos * 8 + 8:(j + 1) * 64, :] = k[jj * 56 + vpos * 8:(jj + 1) * 56, s * 128:(s + 1) * 128]
                if c == 0:
                    cp_wv.wait()
                    wvT = wv_scr[...].astype(f32).T.astype(bf16)
                kb_some(11)
                qt = lax.dot_general(wqT, ln, NT, preferred_element_type=f32) * (DH ** -0.5 * LOG2E)
                qt_scr[c] = pltpu.bitcast(qt.astype(bf16), u32)
                for s in range(4):
                    qf_scr[c * 4 + s] = qt[s * 128:(s + 1) * 128]
                kb_some(11)
                vtf = lax.dot_general(wvT, ln, NT, preferred_element_type=f32)
                va = jnp.max(jnp.abs(vtf).reshape(D // 8, 8, PC), axis=0)
                for n in range(PC // 128):
                    vmax = va[:, n * 128:(n + 1) * 128] if vmax is None else jnp.maximum(vmax, va[:, n * 128:(n + 1) * 128])
                vt = pltpu.bitcast(vtf.astype(bf16), u32)
                for jj in range(PC // TS):
                    vt_scr[c * (PC // TS) + jj] = vt[:, jj * TS:(jj + 1) * TS]
            bad_scr[...] = vmax
            for cp in cp_late:
                cp.wait()

        def block(t, bad):
            gl = [g for g in range(8) if g != vpos]
            stream = [(r, j, g) for r in range(HU) for j in range(NK) for g in reversed(gl)]
            NS = len(stream)
            NC = HU * NK
            cuts = {}
            for c in range(NC):
                cuts.setdefault(min((c + 1) * GM + lag, NS), []).append(c)
            row64 = pl.multiple_of(t * 64, 64)
            row128 = pl.multiple_of(t * 128, 128)
            qz = {}
            def get_qz(r):
                if r not in qz:
                    parts = []
                    if r > 0:
                        parts.append(jnp.zeros((8 * r, TQ), u32))
                    parts.append(qt_scr[i, pl.ds(row64 + 8 * r, 8), :])
                    if r < 7:
                        parts.append(jnp.zeros((8 * (7 - r), TQ), u32))
                    qz[r] = pltpu.bitcast(jnp.concatenate(parts, axis=0), bf16)
                return qz[r]
            P = {}
            l8 = {}
            lv = {}
            acc = {}
            V = {}
            badl = [bad]
            def add_l(r, p):
                for a in (p[0:8], p[8:16]):
                    l8[r] = a if r not in l8 else l8[r] + a
            def vpu_out(c, o):
                r, j = divmod(c, NK)
                n, g2 = divmod(o, 2)
                zc = zs_ref[(c * 8 + o) // share]
                accs = [None] * nacc
                for d in range(DH):
                    kb = kb_scr[t + zc, r * DH + d, j * 16 + g2 * 8:j * 16 + g2 * 8 + 8, :]
                    qb = jnp.broadcast_to(qf_scr[i * 4 + t + zc, r * DH + d:r * DH + d + 1, n * 128:(n + 1) * 128], (8, 128))
                    pr = kb * qb
                    a = d % nacc
                    accs[a] = pr if accs[a] is None else accs[a] + pr
                sv = accs[0]
                for a in accs[1:]:
                    sv = sv + a
                p = jnp.exp2(sv)
                lv[(r, n)] = p if (r, n) not in lv else lv[(r, n)] + p
                V[(c, o)] = p
                return sv
            slots = []
            for pos in range(NS + 1):
                for c in cuts.get(pos, []):
                    slots.append(('pv', c))
                if pos < NS:
                    slots.append(('qk', pos))
            pv_slot = {c: n for n, (k, c) in enumerate(slots) if k == 'pv'}
            sched = {}
            NSL = len(slots)
            for c in range(NC):
                for o in range(8):
                    q = c * 8 + (o // share) * share + share - 1
                    sl = q + off if q + off + taper < NSL else q + max(-2, off - ((q + off + taper - NSL) * (off + 2)) // taper)
                    sched.setdefault(min(max(sl, 1), pv_slot[c] - 1), []).append((c, o))
            def inject(a32, sl):
                deps = [vpu_out(cc, o) for (cc, o) in sched.get(sl, [])]
                if not deps:
                    return a32
                d1 = pltpu.bitcast(deps[0], u32)
                for dd in deps[1:]:
                    d1 = d1 | pltpu.bitcast(dd, u32)
                return a32 | (d1 & z_ref[...])
            def do_pv(c, sl):
                r, j = divmod(c, NK)
                jt, jo = divmod(j * TK, TS)
                vt = pltpu.bitcast(inject(vt_scr[jt, pl.ds(row64 + 8 * r, 8), jo:jo + TK], sl), bf16)
                pvv = jnp.concatenate([jnp.concatenate([V.pop((c, 2 * n)), V.pop((c, 2 * n + 1))], axis=0) for n in range(NL)], axis=1)
                P[(r, j, vpos)] = pvv
                p = jnp.concatenate([P.pop((r, j, g)) for g in range(8)], axis=0).astype(bf16)
                a0 = acc[r] if r in acc else zacc[...]
                acc[r] = a0 + jnp.dot(vt, p, preferred_element_type=f32)
                if j == NK - 1:
                    lt = l8[r] + jnp.concatenate([lv[(r, n)] for n in range(NL)], axis=1)
                    l = jnp.sum(lt, axis=0, keepdims=True)
                    o = acc[r] * (1.0 / l)
                    ot_scr[pl.ds(row128 + DH * r, DH), :] = o
                    if fb:
                        lmin, lmax = badl[0]
                        for n in range(NL):
                            lmin = jnp.minimum(lmin, l[:, n * 128:(n + 1) * 128])
                            lmax = jnp.maximum(lmax, l[:, n * 128:(n + 1) * 128])
                        badl[0] = (lmin, lmax)
            seg = []
            def flush():
                if not seg:
                    return
                r = seg[0][0][0]
                kc = pltpu.bitcast(jnp.concatenate([kk for (_, kk) in seg], axis=0), bf16)
                s = jnp.dot(kc, get_qz(r), preferred_element_type=f32)
                for n, (key, _) in enumerate(seg):
                    p = jnp.exp2(s[n * 16:(n + 1) * 16])
                    add_l(r, p)
                    P[key] = p
                seg.clear()
            for sl, (kind, v) in enumerate(slots):
                if kind == 'pv':
                    flush()
                    do_pv(v, sl)
                else:
                    key = stream[v]
                    if seg and seg[0][0][0] != key[0]:
                        flush()
                    _, j, g = key
                    grp = j * 8 + g
                    seg.append((key, inject(k_scr[t, grp * 8:(grp + 1) * 8, :], sl)))
            flush()
            return badl[0]

        def safe_head(h, carry):
            slab = h // 8
            r = h % 8
            row8 = pl.multiple_of(h * 8, 8)
            qh = qt_scr[i, pl.ds(row8, 8), :]
            z = jnp.zeros_like(qh)
            qz = pltpu.bitcast(jnp.concatenate([jnp.where(r == j, qh, z) for j in range(8)], axis=0), bf16)
            def chunk(j, c):
                m, l, acc = c
                kc = pltpu.bitcast(k_scr[slab, pl.ds(pl.multiple_of(j * (TS // 2), TS // 2), TS // 2), :], bf16)
                s = jnp.dot(kc, qz, preferred_element_type=f32)
                mn = jnp.maximum(m, jnp.max(s, axis=0, keepdims=True))
                a = jnp.exp2(m - mn)
                p = jnp.exp2(s - mn)
                vt = pltpu.bitcast(vt_scr[j, pl.ds(row8, 8), :], bf16)
                l = l * a + jnp.sum(p, axis=0, keepdims=True)
                acc = acc * a + jnp.dot(vt, p.astype(bf16), preferred_element_type=f32)
                return mn, l, acc
            init = (jnp.full((1, TQ), -jnp.inf, f32), jnp.zeros((1, TQ), f32), jnp.zeros((DH, TQ), f32))
            m, l, acc = lax.fori_loop(0, S // TS, chunk, init)
            ot_scr[pl.ds(pl.multiple_of(h * DH, DH), DH), :] = acc / l
            return carry

        with scope('prologue'):
            pl.when(i == 0)(_prologue)
        with scope('attn'):
            one = jnp.full((1, 128), 0.0 if force_fb else 1.0, f32)
            lmin, lmax = lax.fori_loop(0, H // HU, block, (one, one))
        if fb:
            with scope('fb'):
                ok = (lmin >= L_LO) & (lmax <= L_HI) & (bad_scr[...] <= L_HI)
                @pl.when(jnp.max(jnp.where(ok, 0.0, 1.0)) > 0.0)
                def _():
                    lax.fori_loop(0, H, safe_head, 0)

        with scope('epi'):
            o = ot_scr[...].T.astype(bf16)
            xq = x_scr[i].reshape(TQ, D).astype(f32)
            h1 = xq + jnp.dot(o, wo_scr[...], preferred_element_type=f32)
            ln2 = _ln(h1).astype(bf16)
            g = jnp.dot(ln2, w1_scr[...], preferred_element_type=f32) + b1_scr[...].astype(f32).reshape(1, F)
            g = _gelu(g).astype(bf16)
            y = jnp.dot(g, w2_scr[...], preferred_element_type=f32) + b2_scr[...].astype(f32).reshape(1, D)
            o_ref[...] = (h1 + y).astype(o_ref.dtype)

    @jax.jit
    def fn(A_x, A_wqkv, A_wo, B_x, B_w1, B_b1, B_w2, B_b2):
        x = A_x.reshape(NK, TK, D)
        anyspec = pl.BlockSpec(memory_space=pl.ANY)
        out = pl.pallas_call(
            kernel,
            grid=(NQ,),
            in_specs=[anyspec] * 7,
            out_specs=pl.BlockSpec((TQ, D), lambda i: (i, 0)),
            out_shape=jax.ShapeDtypeStruct((S, D), bf16),
            scratch_shapes=[
                pltpu.VMEM((4, PC // TK, TK, D), bf16),
                pltpu.VMEM((NK, 16, D), bf16),
                pltpu.VMEM((D, D), bf16),
                pltpu.VMEM((D, D), bf16),
                pltpu.VMEM((D, D), bf16),
                pltpu.VMEM((D, D), bf16),
                pltpu.VMEM((D, F), bf16),
                pltpu.VMEM((F, D), bf16),
                pltpu.SemaphoreType.DMA((13,)),
                pltpu.VMEM((4, S // 2, 128), u32),
                pltpu.VMEM((4, 128, NK * 16, 128), f32),
                pltpu.VMEM((NQ, D // 2, TQ), u32),
                pltpu.VMEM((NQ * 4, 128, TQ), f32),
                pltpu.VMEM((S // TS, D // 2, TS), u32),
                pltpu.VMEM((D, TQ), f32),
                pltpu.VMEM((DH, TQ), f32),
                pltpu.VMEM((8, 128), u32),
                pltpu.SMEM((NZ,), jnp.int32),
                pltpu.VMEM((8, 128), f32),
                pltpu.VMEM((F,), bf16),
                pltpu.VMEM((D,), bf16),
            ],
            compiler_params=pltpu.CompilerParams(dimension_semantics=("arbitrary",), vmem_limit_bytes=120 * 1024 * 1024),
        )(x, A_wqkv, A_wo, B_w1, B_b1, B_w2, B_b2)
        return out.reshape(1, S, D)
    return fn


_impl = _make()


@jax.jit
def pallas_sequential_preLN__softmax_full_mha__dense_activation_gelu__prompt_kernel(
    A_x: jax.Array,
    A_wqkv: jax.Array,
    A_wo: jax.Array,
    B_x: jax.Array,
    B_w1: jax.Array,
    B_b1: jax.Array,
    B_w2: jax.Array,
    B_b2: jax.Array,
):
    return _impl(A_x, A_wqkv, A_wo, B_x, B_w1, B_b1, B_w2, B_b2)
```

```python
import math

import jax
import jax.numpy as jnp
from jax import lax
import jax.experimental.pallas as pl
import jax.experimental.pallas.tpu as pltpu

S, D, H, DH, F = 2048, 512, 32, 16, 1792
LOG2E = 1.4426950408889634
f32, bf16, u32 = jnp.float32, jnp.bfloat16, jnp.uint32

TQ = 512
TK = 128
NQ = S // TQ
NK = S // TK
NL = TQ // 128
HU = 8
CPC = TQ // TK
TS = 256
E = 10
EH = 2
NZ = HU * NK * NL
L_LO, L_HI, V_HI = 2.0 ** -20, 2.0 ** 90, 2.0 ** 30
NT = (((1,), (1,)), ((), ()))
USTREAM = [(j, g) for j in range(NK) for g in reversed(range(1, 8))]


def _ln(x):
    m = jnp.mean(x, axis=-1, keepdims=True)
    xc = x - m
    v = jnp.mean(xc * xc, axis=-1, keepdims=True)
    return xc * lax.rsqrt(v + 1e-5)


def _gelu(x):
    c = math.sqrt(2.0 / math.pi)
    return 0.5 * x * (1.0 + jnp.tanh(c * (x + 0.044715 * (x * x * x))))


def _pk(x):
    return [pltpu.bitcast(x[:, n * 128:(n + 1) * 128].astype(bf16), u32) for n in range(x.shape[1] // 128)]


def _kernel(x_hbm, wqkv_hbm, wo_hbm, w1_hbm, b1_hbm, w2_hbm, b2_hbm, o_ref,
            x_scr, xv_scr, wq_scr, wk_scr, wv_scr, wo_scr, w1_scr, w2_scr, sems,
            k_scr, kb_scr, qt_scr, qf_scr, vt_scr, ot_scr, pc_scr, zacc, z_ref, zs_ref,
            vmax_scr, lm_scr, b1_scr, b2_scr):
    i = pl.program_id(0)

    def qz_of(ti, row, r):
        parts = []
        if r > 0:
            parts.append(jnp.zeros((8 * r, TQ), u32))
        parts.append(qt_scr[ti, pl.ds(row, 8), :])
        if r < 7:
            parts.append(jnp.zeros((8 * (7 - r), TQ), u32))
        return pltpu.bitcast(jnp.concatenate(parts, axis=0), bf16)

    def prologue():
        cp_xv = pltpu.make_async_copy(x_hbm.at[:, 0:16, :], xv_scr, sems.at[0])
        cp_wk = pltpu.make_async_copy(wqkv_hbm.at[:, D:2 * D], wk_scr, sems.at[1])
        cp_wq = pltpu.make_async_copy(wqkv_hbm.at[:, 0:D], wq_scr, sems.at[2])
        cp_wv = pltpu.make_async_copy(wqkv_hbm.at[:, 2 * D:3 * D], wv_scr, sems.at[3])
        cp_x = [pltpu.make_async_copy(x_hbm.at[c * CPC:(c + 1) * CPC], x_scr.at[c], sems.at[4 + c])
                for c in range(NQ)]
        cp_late = [pltpu.make_async_copy(wo_hbm, wo_scr, sems.at[8]),
                   pltpu.make_async_copy(w1_hbm, w1_scr, sems.at[9]),
                   pltpu.make_async_copy(b1_hbm, b1_scr, sems.at[10]),
                   pltpu.make_async_copy(w2_hbm, w2_scr, sems.at[11]),
                   pltpu.make_async_copy(b2_hbm, b2_scr, sems.at[12])]
        for cp in (cp_xv, cp_wk, cp_x[0], cp_wq, cp_x[1], cp_wv, cp_x[2], cp_x[3]):
            cp.start()
        zacc[...] = jnp.zeros_like(zacc)
        z_ref[...] = jnp.zeros_like(z_ref)
        for n in range(NZ):
            zs_ref[n] = 0

        cp_xv.wait()
        lnv = _ln(xv_scr[...].reshape(NK * 16, D).astype(f32)).astype(bf16)
        cp_wk.wait()
        wk = wk_scr[...]
        kv = _pk(jnp.dot(lnv, wk, preferred_element_type=f32))
        for s in range(4):
            for j in range(NK):
                k_scr[s, j * 64:j * 64 + 8, :] = kv[s][j * 8:(j + 1) * 8]
        work = iter([(c, s) for c in range(128) for s in range(4)])

        def kb_some(n):
            for _ in range(n):
                c, s = next(work)
                b = jnp.broadcast_to(kv[s][:, c:c + 1], (NK * 8, 128))
                kb_scr[s, c] = pltpu.bitcast(b, bf16).astype(f32)

        lnm, lnf, wT, vmax = {}, {}, {}, []

        def do_ln(c):
            m = _ln(jnp.concatenate([x_scr[c, jj, 16:TK, :] for jj in range(CPC)], axis=0).astype(f32)).astype(bf16)
            rows = []
            for jj in range(CPC):
                j = c * CPC + jj
                lnm[j] = m[jj * 112:(jj + 1) * 112]
                rows += [lnv[j * 16:(j + 1) * 16], lnm[j]]
            lnf[c] = jnp.concatenate(rows, axis=0)

        def do_k(j0, j1):
            lhs = jnp.concatenate([lnm[j] for j in range(j0, j1)], axis=0)
            k = _pk(jnp.dot(lhs, wk, preferred_element_type=f32))
            for s in range(4):
                for j in range(j0, j1):
                    k_scr[s, j * 64 + 8:(j + 1) * 64, :] = k[s][(j - j0) * 56:(j - j0 + 1) * 56]

        def do_q(c):
            qt = lax.dot_general(wT['q'], lnf[c], NT, preferred_element_type=f32) * (DH ** -0.5 * LOG2E)
            for n, pk in enumerate(_pk(qt)):
                qt_scr[c, :, n * 128:(n + 1) * 128] = pk
            for s in range(4):
                qf_scr[c * 4 + s] = qt[s * 128:(s + 1) * 128]

        def do_v(c):
            vtf = lax.dot_general(wT['v'], lnf[c], NT, preferred_element_type=f32)
            va = jnp.max(jnp.abs(vtf).reshape(D // 8, 8, TQ), axis=0)
            for n in range(NL):
                vn = va[:, n * 128:(n + 1) * 128]
                vmax[:] = [jnp.maximum(vmax[0], vn) if vmax else vn]
            for n, pk in enumerate(_pk(vtf)):
                jt, jo = divmod(c * TQ + n * 128, TS)
                vt_scr[jt, :, jo:jo + 128] = pk

        kb_some(8)
        cp_x[0].wait()
        do_ln(0)
        do_k(0, 2)
        kb_some(28)
        cp_wq.wait()
        cp_x[1].wait()
        wT['q'] = wq_scr[...].astype(f32).T.astype(bf16)
        do_ln(1)
        do_k(2, 4)
        kb_some(46)
        do_q(0)
        kb_some(46)
        do_k(4, 8)
        cp_wv.wait()
        cp_x[2].wait()
        cp_x[3].wait()
        for cp in cp_late:
            cp.start()
        wT['v'] = wv_scr[...].astype(f32).T.astype(bf16)
        rest = 512 - 8 - 28 - 92
        seq = [lambda: do_q(1), lambda: do_v(0), lambda: do_ln(2), lambda: do_v(1), lambda: do_k(8, 12),
               lambda: do_ln(3), lambda: do_q(2), lambda: do_v(2), lambda: do_k(12, 16), lambda: do_q(3),
               lambda: do_v(3)]
        done = 0
        for n, fn in enumerate(seq):
            fn()
            tgt = min(rest, (rest * (n + 1)) // (len(seq) - 1))
            kb_some(tgt - done)
            done = tgt
        kc = jnp.concatenate([k_scr[0, (j * 8 + g) * 8:(j * 8 + g) * 8 + 8, :] for (j, g) in USTREAM[:E]], axis=0)
        pc_scr[...] = jnp.exp2(jnp.dot(pltpu.bitcast(kc, bf16), qz_of(0, 0, 0), preferred_element_type=f32))
        vmax_scr[...] = vmax[0]
        for cp in cp_late:
            cp.wait()

    def block(t, lrange):
        NU = len(USTREAM)
        full = [(r, j, g) for r in range(HU + 1) for (j, g) in USTREAM]
        slots = []
        for pos, key in enumerate(full[E:E + HU * NU]):
            slots.append(('qk', key))
            if pos % 7 == 6:
                slots.append(('pv', divmod(pos // 7, NK)))
        sched = {}
        for c in range(HU * NK):
            for n in range(NL):
                sched[max(c * 8 + 2 * n, 1 + n if c == 0 else 0)] = (c, n)
        row64 = pl.multiple_of(t * 64, 64)
        row128 = pl.multiple_of(t * 128, 128)
        tn = (t + 1) % 4
        inx = jnp.minimum(i + (t + 1) // 4, NQ - 1)
        qbase = i * 4 + t
        qz, P, V, lsum, acc = {}, {}, {}, {}, {}
        lr = list(lrange)

        def get_qz(r):
            if r not in qz:
                qz[r] = qz_of(i, row64 + 8 * r, r) if r < HU else qz_of(inx, pl.multiple_of(tn * 64, 64), 0)
            return qz[r]

        def add_l(key, p):
            for a in (p[0:8], p[8:16]):
                lsum[key] = a if key not in lsum else lsum[key] + a

        def paced(a32, sl):
            if sl not in sched:
                return a32
            c, n = sched[sl]
            r, j = divmod(c, NK)
            zc = zs_ref[c * NL + n]
            kref = kb_scr.at[t + zc]
            qref = qf_scr.at[qbase + zc]
            sv = None
            for d in range(r * DH, (r + 1) * DH):
                pr = kref[d, j * 16:j * 16 + 16, :] * qref[d:d + 1, n * 128:(n + 1) * 128]
                sv = pr if sv is None else sv + pr
            p = jnp.exp2(sv)
            add_l((r, n), p)
            V[(c, n)] = p
            s32 = pltpu.bitcast(sv, u32)
            return a32 | ((s32[0:8] | s32[8:16]) & z_ref[...])

        def do_pv(r, j, sl):
            jt, jo = divmod(j * TK, TS)
            vt = pltpu.bitcast(paced(vt_scr[jt, pl.ds(row64 + 8 * r, 8), jo:jo + TK], sl), bf16)
            P[(r, j, 0)] = jnp.concatenate([V.pop((r * NK + j, n)) for n in range(NL)], axis=1)
            p = jnp.concatenate([P.pop((r, j, g)) for g in range(8)], axis=0).astype(bf16)
            a0 = acc[r] if r in acc else zacc[...]
            acc[r] = a0 + jnp.dot(vt, p, preferred_element_type=f32)
            if j == NK - 1:
                lt = lsum[r] + jnp.concatenate([lsum[(r, n)] for n in range(NL)], axis=1)
                l = jnp.sum(lt, axis=0, keepdims=True)
                inv = pl.reciprocal(l, approx=True)
                inv = inv * (2.0 - l * inv)
                ot_scr[pl.ds(row128 + DH * r, DH), :] = acc[r] * inv
                for n in range(NL):
                    lr[0] = jnp.minimum(lr[0], l[:, n * 128:(n + 1) * 128])
                    lr[1] = jnp.maximum(lr[1], l[:, n * 128:(n + 1) * 128])

        for n, key in enumerate(full[:E]):
            P[key] = pc_scr[n * 16:(n + 1) * 16, :]
            add_l(0, P[key])
        seg = []

        def flush():
            if not seg:
                return
            r = seg[0][0][0]
            kc = pltpu.bitcast(jnp.concatenate([kk for (_, kk) in seg], axis=0), bf16)
            pe = jnp.exp2(jnp.dot(kc, get_qz(r), preferred_element_type=f32))
            for n, (key, _) in enumerate(seg):
                p = pe[n * 16:(n + 1) * 16]
                if r < HU:
                    add_l(r, p)
                    P[key] = p
                else:
                    m = USTREAM.index(key[1:])
                    pc_scr[m * 16:(m + 1) * 16, :] = p
            seg.clear()

        for sl, (kind, key) in enumerate(slots):
            if kind == 'pv':
                flush()
                do_pv(key[0], key[1], sl)
            else:
                if seg and seg[0][0][0] != key[0]:
                    flush()
                r, j, g = key
                grp = j * 8 + g
                seg.append((key, paced(k_scr[t if r < HU else tn, grp * 8:(grp + 1) * 8, :], sl)))
        return tuple(lr)

    def safe_head(h, carry):
        slab = h // 8
        r = h % 8
        row8 = pl.multiple_of(h * 8, 8)
        qh = qt_scr[i, pl.ds(row8, 8), :]
        z = jnp.zeros_like(qh)
        qz = pltpu.bitcast(jnp.concatenate([jnp.where(r == n, qh, z) for n in range(8)], axis=0), bf16)

        def chunk(j, c):
            m, l, acc = c
            kc = pltpu.bitcast(k_scr[slab, pl.ds(pl.multiple_of(j * (TS // 2), TS // 2), TS // 2), :], bf16)
            s = jnp.dot(kc, qz, preferred_element_type=f32)
            mn = jnp.maximum(m, jnp.max(s, axis=0, keepdims=True))
            a = jnp.exp2(m - mn)
            p = jnp.exp2(s - mn)
            vt = pltpu.bitcast(vt_scr[j, pl.ds(row8, 8), :], bf16)
            l = l * a + jnp.sum(p, axis=0, keepdims=True)
            acc = acc * a + jnp.dot(vt, p.astype(bf16), preferred_element_type=f32)
            return mn, l, acc

        init = (jnp.full((1, TQ), -jnp.inf, f32), jnp.zeros((1, TQ), f32), jnp.zeros((DH, TQ), f32))
        _, l, acc = lax.fori_loop(0, S // TS, chunk, init)
        ot_scr[pl.ds(pl.multiple_of(h * DH, DH), DH), :] = acc / l
        return carry

    def epilogue(c):
        attempt, _ = c

        @pl.when(attempt == 1)
        def _():
            lax.fori_loop(0, H, safe_head, 0)

        HR = TQ // EH
        b1 = b1_scr[...].astype(f32).reshape(1, F)
        b2 = b2_scr[...].astype(f32).reshape(1, D)
        h1 = []
        for e in range(EH):
            o = ot_scr[:, e * HR:(e + 1) * HR].T.astype(bf16)
            xq = x_scr[i, e * (HR // TK):(e + 1) * (HR // TK)].reshape(HR, D).astype(f32)
            h1.append(xq + jnp.dot(o, wo_scr[...], preferred_element_type=f32))
        gs = []
        for e in range(EH):
            ln2 = _ln(h1[e]).astype(bf16)
            gs.append(_gelu(jnp.dot(ln2, w1_scr[...], preferred_element_type=f32) + b1).astype(bf16))
        ok = (lm_scr[0:1, :] >= L_LO) & (lm_scr[1:2, :] <= L_HI) & (vmax_scr[...] <= V_HI)
        nbad = jnp.max(jnp.where(ok, 0, 1))
        for e in range(EH):
            y = jnp.dot(gs[e], w2_scr[...], preferred_element_type=f32) + b2
            o_ref[e * HR:(e + 1) * HR, :] = (h1[e] + y).astype(o_ref.dtype)
        return attempt + 1, 1 + nbad

    pl.when(i == 0)(prologue)
    one = jnp.ones((1, 128), f32)
    lmin, lmax = lax.fori_loop(0, H // HU, block, (one, one))
    lm_scr[0:1, :] = lmin
    lm_scr[1:2, :] = lmax
    lax.while_loop(lambda c: c[0] < c[1], epilogue, (jnp.int32(0), jnp.int32(1)))


@jax.jit
def pallas_sequential_preLN__softmax_full_mha__dense_activation_gelu__prompt_kernel(
    A_x: jax.Array,
    A_wqkv: jax.Array,
    A_wo: jax.Array,
    B_x: jax.Array,
    B_w1: jax.Array,
    B_b1: jax.Array,
    B_w2: jax.Array,
    B_b2: jax.Array,
):
    del B_x
    hbm = pl.BlockSpec(memory_space=pl.ANY)
    out = pl.pallas_call(
        _kernel,
        grid=(NQ,),
        in_specs=[hbm] * 7,
        out_specs=pl.BlockSpec((TQ, D), lambda i: (i, 0)),
        out_shape=jax.ShapeDtypeStruct((S, D), bf16),
        scratch_shapes=[
            pltpu.VMEM((NQ, CPC, TK, D), bf16),
            pltpu.VMEM((NK, 16, D), bf16),
            pltpu.VMEM((D, D), bf16),
            pltpu.VMEM((D, D), bf16),
            pltpu.VMEM((D, D), bf16),
            pltpu.VMEM((D, D), bf16),
            pltpu.VMEM((D, F), bf16),
            pltpu.VMEM((F, D), bf16),
            pltpu.SemaphoreType.DMA((13,)),
            pltpu.VMEM((4, S // 2, 128), u32),
            pltpu.VMEM((4, 128, NK * 16, 128), f32),
            pltpu.VMEM((NQ, D // 2, TQ), u32),
            pltpu.VMEM((NQ * 4, 128, TQ), f32),
            pltpu.VMEM((S // TS, D // 2, TS), u32),
            pltpu.VMEM((D, TQ), f32),
            pltpu.VMEM((E * 16, TQ), f32),
            pltpu.VMEM((DH, TQ), f32),
            pltpu.VMEM((8, 128), u32),
            pltpu.SMEM((NZ,), jnp.int32),
            pltpu.VMEM((8, 128), f32),
            pltpu.VMEM((8, 128), f32),
            pltpu.VMEM((F,), bf16),
            pltpu.VMEM((D,), bf16),
        ],
        compiler_params=pltpu.CompilerParams(
            dimension_semantics=("arbitrary",), vmem_limit_bytes=120 * 1024 * 1024),
    )(A_x.reshape(NK, TK, D), A_wqkv, A_wo, B_w1, B_b1, B_w2, B_b2)
    return out.reshape(1, S, D)
```

```python
import math

import jax
import jax.numpy as jnp
from jax import lax
import jax.experimental.pallas as pl
import jax.experimental.pallas.tpu as pltpu

S, D, H, DH, F = 2048, 512, 32, 16, 1792
LOG2E = 1.4426950408889634
f32, bf16, u32 = jnp.float32, jnp.bfloat16, jnp.uint32

TQ = 512
TK = 128
NQ = S // TQ
NK = S // TK
NL = TQ // 128
HU = 8
CPC = TQ // TK
TS = 256
E = 10
EH = 4
HR = TQ // EH
NZ = HU * NK * NL
L_LO, L_HI, V_HI = 2.0 ** -20, 2.0 ** 90, 2.0 ** 30
NT = (((1,), (1,)), ((), ()))
USTREAM = [(j, g) for j in range(NK) for g in reversed(range(1, 8))]


def _ln(x):
    m = jnp.mean(x, axis=-1, keepdims=True)
    xc = x - m
    v = jnp.mean(xc * xc, axis=-1, keepdims=True)
    return xc * lax.rsqrt(v + 1e-5)


def _gelu(x):
    c = math.sqrt(2.0 / math.pi)
    return 0.5 * x * (1.0 + jnp.tanh(c * (x + 0.044715 * (x * x * x))))


def _pk(x):
    return [pltpu.bitcast(x[:, n * 128:(n + 1) * 128].astype(bf16), u32) for n in range(x.shape[1] // 128)]


def _kernel(x_hbm, wqkv_hbm, wo_hbm, w1_hbm, b1_hbm, w2_hbm, b2_hbm, o_hbm,
            x_scr, xv_scr, wq_scr, wk_scr, wv_scr, wo_scr, w1_scr, w2_scr, sems,
            k_scr, kb_scr, qt_scr, qf_scr, vt_scr, ot_scr, pc_scr, zacc, z_ref, zs_ref,
            vmax_scr, lm_scr, os_scr, osems, b1_scr, b2_scr):
    i = pl.program_id(0)

    def qz_of(ti, row, r):
        parts = []
        if r > 0:
            parts.append(jnp.zeros((8 * r, TQ), u32))
        parts.append(qt_scr[ti, pl.ds(row, 8), :])
        if r < 7:
            parts.append(jnp.zeros((8 * (7 - r), TQ), u32))
        return pltpu.bitcast(jnp.concatenate(parts, axis=0), bf16)

    def prologue():
        cp_xv = pltpu.make_async_copy(x_hbm.at[:, 0:16, :], xv_scr, sems.at[0])
        cp_wk = pltpu.make_async_copy(wqkv_hbm.at[:, D:2 * D], wk_scr, sems.at[1])
        cp_wq = pltpu.make_async_copy(wqkv_hbm.at[:, 0:D], wq_scr, sems.at[2])
        cp_wv = pltpu.make_async_copy(wqkv_hbm.at[:, 2 * D:3 * D], wv_scr, sems.at[3])
        cp_x = [pltpu.make_async_copy(x_hbm.at[c * CPC:(c + 1) * CPC], x_scr.at[c], sems.at[4 + c])
                for c in range(NQ)]
        cp_late = [pltpu.make_async_copy(wo_hbm, wo_scr, sems.at[8]),
                   pltpu.make_async_copy(w1_hbm, w1_scr, sems.at[9]),
                   pltpu.make_async_copy(b1_hbm, b1_scr, sems.at[10]),
                   pltpu.make_async_copy(w2_hbm, w2_scr, sems.at[11]),
                   pltpu.make_async_copy(b2_hbm, b2_scr, sems.at[12])]
        for cp in (cp_xv, cp_wk, cp_x[0], cp_wq, cp_x[1], cp_wv, cp_x[2], cp_x[3]):
            cp.start()
        zacc[...] = jnp.zeros_like(zacc)
        z_ref[...] = jnp.zeros_like(z_ref)
        for n in range(NZ):
            zs_ref[n] = 0

        cp_xv.wait()
        lnv = _ln(xv_scr[...].reshape(NK * 16, D).astype(f32)).astype(bf16)
        cp_wk.wait()
        wk = wk_scr[...]
        kv = _pk(jnp.dot(lnv, wk, preferred_element_type=f32))
        for s in range(4):
            for j in range(NK):
                k_scr[s, j * 64:j * 64 + 8, :] = kv[s][j * 8:(j + 1) * 8]
        work = iter([(c, s) for c in range(128) for s in range(4)])

        def kb_some(n):
            for _ in range(n):
                c, s = next(work)
                b = jnp.broadcast_to(kv[s][:, c:c + 1], (NK * 8, 128))
                kb_scr[s, c] = pltpu.bitcast(b, bf16).astype(f32)

        lnm, lnf, wT, vmax = {}, {}, {}, []

        def do_ln(c):
            m = _ln(jnp.concatenate([x_scr[c, jj, 16:TK, :] for jj in range(CPC)], axis=0).astype(f32)).astype(bf16)
            rows = []
            for jj in range(CPC):
                j = c * CPC + jj
                lnm[j] = m[jj * 112:(jj + 1) * 112]
                rows += [lnv[j * 16:(j + 1) * 16], lnm[j]]
            lnf[c] = jnp.concatenate(rows, axis=0)

        def do_k(j0, j1):
            lhs = jnp.concatenate([lnm[j] for j in range(j0, j1)], axis=0)
            k = _pk(jnp.dot(lhs, wk, preferred_element_type=f32))
            for s in range(4):
                for j in range(j0, j1):
                    k_scr[s, j * 64 + 8:(j + 1) * 64, :] = k[s][(j - j0) * 56:(j - j0 + 1) * 56]

        def do_q(c):
            qt = lax.dot_general(wT['q'], lnf[c], NT, preferred_element_type=f32) * (DH ** -0.5 * LOG2E)
            for n, pk in enumerate(_pk(qt)):
                qt_scr[c, :, n * 128:(n + 1) * 128] = pk
            for s in range(4):
                qf_scr[c * 4 + s] = qt[s * 128:(s + 1) * 128]

        def do_v(c):
            vtf = lax.dot_general(wT['v'], lnf[c], NT, preferred_element_type=f32)
            va = jnp.max(jnp.abs(vtf).reshape(D // 8, 8, TQ), axis=0)
            for n in range(NL):
                vn = va[:, n * 128:(n + 1) * 128]
                vmax[:] = [jnp.maximum(vmax[0], vn) if vmax else vn]
            for n, pk in enumerate(_pk(vtf)):
                jt, jo = divmod(c * TQ + n * 128, TS)
                vt_scr[jt, :, jo:jo + 128] = pk

        kb_some(8)
        cp_x[0].wait()
        do_ln(0)
        do_k(0, 2)
        kb_some(28)
        cp_wq.wait()
        cp_x[1].wait()
        wT['q'] = wq_scr[...].astype(f32).T.astype(bf16)
        do_ln(1)
        do_k(2, 4)
        kb_some(46)
        do_q(0)
        kb_some(46)
        do_k(4, 8)
        cp_wv.wait()
        cp_x[2].wait()
        cp_x[3].wait()
        for cp in cp_late:
            cp.start()
        wT['v'] = wv_scr[...].astype(f32).T.astype(bf16)
        rest = 512 - 8 - 28 - 92
        seq = [lambda: do_q(1), lambda: do_v(0), lambda: do_ln(2), lambda: do_v(1), lambda: do_k(8, 12),
               lambda: do_ln(3), lambda: do_q(2), lambda: do_v(2), lambda: do_k(12, 16), lambda: do_q(3),
               lambda: do_v(3)]
        done = 0
        for n, fn in enumerate(seq):
            fn()
            tgt = min(rest, (rest * (n + 1)) // (len(seq) - 1))
            kb_some(tgt - done)
            done = tgt
        kc = jnp.concatenate([k_scr[0, (j * 8 + g) * 8:(j * 8 + g) * 8 + 8, :] for (j, g) in USTREAM[:E]], axis=0)
        pc_scr[...] = jnp.exp2(jnp.dot(pltpu.bitcast(kc, bf16), qz_of(0, 0, 0), preferred_element_type=f32))
        vmax_scr[...] = vmax[0]
        for cp in cp_late:
            cp.wait()

    def block(t, lrange):
        NU = len(USTREAM)
        full = [(r, j, g) for r in range(HU + 1) for (j, g) in USTREAM]
        slots = []
        for pos, key in enumerate(full[E:E + HU * NU]):
            slots.append(('qk', key))
            if pos % 7 == 6:
                slots.append(('pv', divmod(pos // 7, NK)))
        sched = {}
        for c in range(HU * NK):
            for n in range(NL):
                sched[max(c * 8 + 2 * n, 1 + n if c == 0 else 0)] = (c, n)
        row64 = pl.multiple_of(t * 64, 64)
        row128 = pl.multiple_of(t * 128, 128)
        tn = (t + 1) % 4
        inx = jnp.minimum(i + (t + 1) // 4, NQ - 1)
        qbase = i * 4 + t
        qz, P, V, lsum, acc = {}, {}, {}, {}, {}
        lr = list(lrange)

        def get_qz(r):
            if r not in qz:
                qz[r] = qz_of(i, row64 + 8 * r, r) if r < HU else qz_of(inx, pl.multiple_of(tn * 64, 64), 0)
            return qz[r]

        def add_l(key, p):
            for a in (p[0:8], p[8:16]):
                lsum[key] = a if key not in lsum else lsum[key] + a

        def paced(a32, sl):
            if sl not in sched:
                return a32
            c, n = sched[sl]
            r, j = divmod(c, NK)
            zc = zs_ref[c * NL + n]
            kref = kb_scr.at[t + zc]
            qref = qf_scr.at[qbase + zc]
            sv = None
            for d in range(r * DH, (r + 1) * DH):
                pr = kref[d, j * 16:j * 16 + 16, :] * qref[d:d + 1, n * 128:(n + 1) * 128]
                sv = pr if sv is None else sv + pr
            p = jnp.exp2(sv)
            add_l((r, n), p)
            V[(c, n)] = p
            s32 = pltpu.bitcast(sv, u32)
            return a32 | ((s32[0:8] | s32[8:16]) & z_ref[...])

        def do_pv(r, j, sl):
            jt, jo = divmod(j * TK, TS)
            vt = pltpu.bitcast(paced(vt_scr[jt, pl.ds(row64 + 8 * r, 8), jo:jo + TK], sl), bf16)
            P[(r, j, 0)] = jnp.concatenate([V.pop((r * NK + j, n)) for n in range(NL)], axis=1)
            p = jnp.concatenate([P.pop((r, j, g)) for g in range(8)], axis=0).astype(bf16)
            a0 = acc[r] if r in acc else zacc[...]
            acc[r] = a0 + jnp.dot(vt, p, preferred_element_type=f32)
            if j == NK - 1:
                lt = lsum[r] + jnp.concatenate([lsum[(r, n)] for n in range(NL)], axis=1)
                l = jnp.sum(lt, axis=0, keepdims=True)
                inv = pl.reciprocal(l, approx=True)
                inv = inv * (2.0 - l * inv)
                ot_scr[pl.ds(row128 + DH * r, DH), :] = acc[r] * inv
                for n in range(NL):
                    lr[0] = jnp.minimum(lr[0], l[:, n * 128:(n + 1) * 128])
                    lr[1] = jnp.maximum(lr[1], l[:, n * 128:(n + 1) * 128])

        for n, key in enumerate(full[:E]):
            P[key] = pc_scr[n * 16:(n + 1) * 16, :]
            add_l(0, P[key])
        seg = []

        def flush():
            if not seg:
                return
            r = seg[0][0][0]
            kc = pltpu.bitcast(jnp.concatenate([kk for (_, kk) in seg], axis=0), bf16)
            pe = jnp.exp2(jnp.dot(kc, get_qz(r), preferred_element_type=f32))
            for n, (key, _) in enumerate(seg):
                p = pe[n * 16:(n + 1) * 16]
                if r < HU:
                    add_l(r, p)
                    P[key] = p
                else:
                    m = USTREAM.index(key[1:])
                    pc_scr[m * 16:(m + 1) * 16, :] = p
            seg.clear()

        for sl, (kind, key) in enumerate(slots):
            if kind == 'pv':
                flush()
                do_pv(key[0], key[1], sl)
            else:
                if seg and seg[0][0][0] != key[0]:
                    flush()
                r, j, g = key
                grp = j * 8 + g
                seg.append((key, paced(k_scr[t if r < HU else tn, grp * 8:(grp + 1) * 8, :], sl)))
        return tuple(lr)

    def safe_head(h, carry):
        slab = h // 8
        r = h % 8
        row8 = pl.multiple_of(h * 8, 8)
        qh = qt_scr[i, pl.ds(row8, 8), :]
        z = jnp.zeros_like(qh)
        qz = pltpu.bitcast(jnp.concatenate([jnp.where(r == n, qh, z) for n in range(8)], axis=0), bf16)

        def chunk(j, c):
            m, l, acc = c
            kc = pltpu.bitcast(k_scr[slab, pl.ds(pl.multiple_of(j * (TS // 2), TS // 2), TS // 2), :], bf16)
            s = jnp.dot(kc, qz, preferred_element_type=f32)
            mn = jnp.maximum(m, jnp.max(s, axis=0, keepdims=True))
            a = jnp.exp2(m - mn)
            p = jnp.exp2(s - mn)
            vt = pltpu.bitcast(vt_scr[j, pl.ds(row8, 8), :], bf16)
            l = l * a + jnp.sum(p, axis=0, keepdims=True)
            acc = acc * a + jnp.dot(vt, p.astype(bf16), preferred_element_type=f32)
            return mn, l, acc

        init = (jnp.full((1, TQ), -jnp.inf, f32), jnp.zeros((1, TQ), f32), jnp.zeros((DH, TQ), f32))
        _, l, acc = lax.fori_loop(0, S // TS, chunk, init)
        ot_scr[pl.ds(pl.multiple_of(h * DH, DH), DH), :] = acc / l
        return carry

    def out_cp(e):
        row = pl.multiple_of(i * TQ + e * HR, HR)
        return pltpu.make_async_copy(os_scr.at[e * HR:(e + 1) * HR], o_hbm.at[pl.ds(row, HR)], osems.at[e])

    def epilogue(c):
        attempt, _ = c

        @pl.when(attempt == 1)
        def _():
            lax.fori_loop(0, H, safe_head, 0)

        @pl.when(i + attempt > 0)
        def _():
            for e in range(EH):
                out_cp(e).wait()

        b1 = b1_scr[...].astype(f32).reshape(1, F)
        b2 = b2_scr[...].astype(f32).reshape(1, D)
        h1 = []
        for e in range(EH):
            o = ot_scr[:, e * HR:(e + 1) * HR].T.astype(bf16)
            xq = x_scr[i, e * (HR // TK):(e + 1) * (HR // TK)].reshape(HR, D).astype(f32)
            h1.append(xq + jnp.dot(o, wo_scr[...], preferred_element_type=f32))
        gs = []
        for e in range(EH):
            ln2 = _ln(h1[e]).astype(bf16)
            gs.append(_gelu(jnp.dot(ln2, w1_scr[...], preferred_element_type=f32) + b1).astype(bf16))
        ok = (lm_scr[0:1, :] >= L_LO) & (lm_scr[1:2, :] <= L_HI) & (vmax_scr[...] <= V_HI)
        nbad = jnp.max(jnp.where(ok, 0, 1))
        for e in range(EH):
            y = jnp.dot(gs[e], w2_scr[...], preferred_element_type=f32) + b2
            os_scr[e * HR:(e + 1) * HR, :] = (h1[e] + y).astype(bf16)
            out_cp(e).start()
        return attempt + 1, 1 + nbad

    pl.when(i == 0)(prologue)
    one = jnp.ones((1, 128), f32)
    lmin, lmax = lax.fori_loop(0, H // HU, block, (one, one))
    lm_scr[0:1, :] = lmin
    lm_scr[1:2, :] = lmax
    lax.while_loop(lambda c: c[0] < c[1], epilogue, (jnp.int32(0), jnp.int32(1)))

    @pl.when(i == NQ - 1)
    def _():
        for e in range(EH):
            out_cp(e).wait()


@jax.jit
def pallas_sequential_preLN__softmax_full_mha__dense_activation_gelu__prompt_kernel(
    A_x: jax.Array,
    A_wqkv: jax.Array,
    A_wo: jax.Array,
    B_x: jax.Array,
    B_w1: jax.Array,
    B_b1: jax.Array,
    B_w2: jax.Array,
    B_b2: jax.Array,
):
    del B_x
    hbm = pl.BlockSpec(memory_space=pl.ANY)
    out = pl.pallas_call(
        _kernel,
        grid=(NQ,),
        in_specs=[hbm] * 7,
        out_specs=hbm,
        out_shape=jax.ShapeDtypeStruct((S, D), bf16),
        scratch_shapes=[
            pltpu.VMEM((NQ, CPC, TK, D), bf16),
            pltpu.VMEM((NK, 16, D), bf16),
            pltpu.VMEM((D, D), bf16),
            pltpu.VMEM((D, D), bf16),
            pltpu.VMEM((D, D), bf16),
            pltpu.VMEM((D, D), bf16),
            pltpu.VMEM((D, F), bf16),
            pltpu.VMEM((F, D), bf16),
            pltpu.SemaphoreType.DMA((13,)),
            pltpu.VMEM((4, S // 2, 128), u32),
            pltpu.VMEM((4, 128, NK * 16, 128), f32),
            pltpu.VMEM((NQ, D // 2, TQ), u32),
            pltpu.VMEM((NQ * 4, 128, TQ), f32),
            pltpu.VMEM((S // TS, D // 2, TS), u32),
            pltpu.VMEM((D, TQ), f32),
            pltpu.VMEM((E * 16, TQ), f32),
            pltpu.VMEM((DH, TQ), f32),
            pltpu.VMEM((8, 128), u32),
            pltpu.SMEM((NZ,), jnp.int32),
            pltpu.VMEM((8, 128), f32),
            pltpu.VMEM((8, 128), f32),
            pltpu.VMEM((TQ, D), bf16),
            pltpu.SemaphoreType.DMA((EH,)),
            pltpu.VMEM((F,), bf16),
            pltpu.VMEM((D,), bf16),
        ],
        compiler_params=pltpu.CompilerParams(
            dimension_semantics=("arbitrary",), vmem_limit_bytes=120 * 1024 * 1024),
    )(A_x.reshape(NK, TK, D), A_wqkv, A_wo, B_w1, B_b1, B_w2, B_b2)
    return out.reshape(1, S, D)
```

```python
import math

import jax
import jax.numpy as jnp
from jax import lax
import jax.experimental.pallas as pl
import jax.experimental.pallas.tpu as pltpu

S, D, H, DH, F = 2048, 512, 32, 16, 1792
LOG2E = 1.4426950408889634
f32, bf16, u32 = jnp.float32, jnp.bfloat16, jnp.uint32

TQ = 512
TK = 128
NQ = S // TQ
NK = S // TK
NL = TQ // 128
HU = 8
CPC = TQ // TK
TS = 256
E = 10
EH = 4
HR = TQ // EH
NZ = HU * NK * NL
L_LO, L_HI, V_HI = 2.0 ** -20, 2.0 ** 90, 2.0 ** 30
NT = (((1,), (1,)), ((), ()))
USTREAM = [(j, g) for j in range(NK) for g in reversed(range(1, 8))]


def _ln(x):
    m = jnp.mean(x, axis=-1, keepdims=True)
    xc = x - m
    v = jnp.mean(xc * xc, axis=-1, keepdims=True)
    return xc * lax.rsqrt(v + 1e-5)


def _gelu(x):
    c = math.sqrt(2.0 / math.pi)
    return 0.5 * x * (1.0 + jnp.tanh(c * (x + 0.044715 * (x * x * x))))


def _pk(x):
    return [pltpu.bitcast(x[:, n * 128:(n + 1) * 128].astype(bf16), u32) for n in range(x.shape[1] // 128)]


def _kernel(x_hbm, wqkv_hbm, wo_hbm, w1_hbm, b1_hbm, w2_hbm, b2_hbm, o_hbm,
            x_scr, xv_scr, wq_scr, wk_scr, wv_scr, wo_scr, w1_scr, w2_scr, sems,
            k_scr, kb_scr, qt_scr, qf_scr, vt_scr, ot_scr, pc_scr, zacc, z_ref, zs_ref,
            vmax_scr, lm_scr, os_scr, osems, b1_scr, b2_scr):
    i = pl.program_id(0)

    def qz_of(ti, row, r):
        parts = []
        if r > 0:
            parts.append(jnp.zeros((8 * r, TQ), u32))
        parts.append(qt_scr[ti, pl.ds(row, 8), :])
        if r < 7:
            parts.append(jnp.zeros((8 * (7 - r), TQ), u32))
        return pltpu.bitcast(jnp.concatenate(parts, axis=0), bf16)

    def prologue():
        cp_xv = pltpu.make_async_copy(x_hbm.at[:, 0:16, :], xv_scr, sems.at[0])
        cp_wk = pltpu.make_async_copy(wqkv_hbm.at[:, D:2 * D], wk_scr, sems.at[1])
        cp_wq = pltpu.make_async_copy(wqkv_hbm.at[:, 0:D], wq_scr, sems.at[2])
        cp_wv = pltpu.make_async_copy(wqkv_hbm.at[:, 2 * D:3 * D], wv_scr, sems.at[3])
        cp_x = [pltpu.make_async_copy(x_hbm.at[c * CPC:(c + 1) * CPC], x_scr.at[c], sems.at[4 + c])
                for c in range(NQ)]
        cp_late = [pltpu.make_async_copy(wo_hbm, wo_scr, sems.at[8]),
                   pltpu.make_async_copy(w1_hbm, w1_scr, sems.at[9]),
                   pltpu.make_async_copy(b1_hbm, b1_scr, sems.at[10]),
                   pltpu.make_async_copy(w2_hbm, w2_scr, sems.at[11]),
                   pltpu.make_async_copy(b2_hbm, b2_scr, sems.at[12])]
        for cp in (cp_xv, cp_wk, cp_x[0], cp_wq, cp_x[1], cp_wv, cp_x[2], cp_x[3]):
            cp.start()
        zacc[...] = jnp.zeros_like(zacc)
        z_ref[...] = jnp.zeros_like(z_ref)

        def zero_zs(n, c):
            zs_ref[n] = 0
            return c

        lax.fori_loop(0, NZ, zero_zs, 0, unroll=True)

        cp_xv.wait()
        lnv = _ln(xv_scr[...].reshape(NK * 16, D).astype(f32)).astype(bf16)
        cp_wk.wait()
        wk = wk_scr[...]
        kv = _pk(jnp.dot(lnv, wk, preferred_element_type=f32))
        for s in range(4):
            for j in range(NK):
                k_scr[s, j * 64:j * 64 + 8, :] = kv[s][j * 8:(j + 1) * 8]
        work = iter([(c, s) for c in range(128) for s in range(4)])

        def kb_some(n):
            for _ in range(n):
                c, s = next(work)
                b = jnp.broadcast_to(kv[s][:, c:c + 1], (NK * 8, 128))
                kb_scr[s, c] = pltpu.bitcast(b, bf16).astype(f32)

        lnm, lnf, wT, vmax = {}, {}, {}, []

        def do_ln(c):
            m = _ln(jnp.concatenate([x_scr[c, jj, 16:TK, :] for jj in range(CPC)], axis=0).astype(f32)).astype(bf16)
            rows = []
            for jj in range(CPC):
                j = c * CPC + jj
                lnm[j] = m[jj * 112:(jj + 1) * 112]
                rows += [lnv[j * 16:(j + 1) * 16], lnm[j]]
            lnf[c] = jnp.concatenate(rows, axis=0)

        def do_k(j0, j1):
            lhs = jnp.concatenate([lnm[j] for j in range(j0, j1)], axis=0)
            k = _pk(jnp.dot(lhs, wk, preferred_element_type=f32))
            for s in range(4):
                for j in range(j0, j1):
                    k_scr[s, j * 64 + 8:(j + 1) * 64, :] = k[s][(j - j0) * 56:(j - j0 + 1) * 56]

        def do_q(c):
            qt = lax.dot_general(wT['q'], lnf[c], NT, preferred_element_type=f32) * (DH ** -0.5 * LOG2E)
            for n, pk in enumerate(_pk(qt)):
                qt_scr[c, :, n * 128:(n + 1) * 128] = pk
            for s in range(4):
                qf_scr[c * 4 + s] = qt[s * 128:(s + 1) * 128]

        def do_v(c):
            vtf = lax.dot_general(wT['v'], lnf[c], NT, preferred_element_type=f32)
            va = jnp.max(jnp.abs(vtf).reshape(D // 8, 8, TQ), axis=0)
            for n in range(NL):
                vn = va[:, n * 128:(n + 1) * 128]
                vmax[:] = [jnp.maximum(vmax[0], vn) if vmax else vn]
            for n, pk in enumerate(_pk(vtf)):
                jt, jo = divmod(c * TQ + n * 128, TS)
                vt_scr[jt, :, jo:jo + 128] = pk

        kb_some(8)
        cp_x[0].wait()
        do_ln(0)
        do_k(0, 2)
        kb_some(28)
        cp_wq.wait()
        cp_x[1].wait()
        wT['q'] = wq_scr[...].astype(f32).T.astype(bf16)
        do_ln(1)
        do_k(2, 4)
        kb_some(46)
        do_q(0)
        kb_some(46)
        do_k(4, 8)
        cp_wv.wait()
        cp_x[2].wait()
        cp_x[3].wait()
        for cp in cp_late:
            cp.start()
        wT['v'] = wv_scr[...].astype(f32).T.astype(bf16)
        rest = 512 - 8 - 28 - 92
        seq = [lambda: do_q(1), lambda: do_v(0), lambda: do_ln(2), lambda: do_v(1), lambda: do_k(8, 12),
               lambda: do_ln(3), lambda: do_q(2), lambda: do_v(2), lambda: do_k(12, 16), lambda: do_q(3),
               lambda: do_v(3)]
        done = 0
        for n, fn in enumerate(seq):
            fn()
            tgt = min(rest, (rest * (n + 1)) // (len(seq) - 1))
            kb_some(tgt - done)
            done = tgt
        kc = jnp.concatenate([k_scr[0, (j * 8 + g) * 8:(j * 8 + g) * 8 + 8, :] for (j, g) in USTREAM[:E]], axis=0)
        pc_scr[...] = jnp.exp2(jnp.dot(pltpu.bitcast(kc, bf16), qz_of(0, 0, 0), preferred_element_type=f32))
        vmax_scr[...] = vmax[0]
        for cp in cp_late:
            cp.wait()

    def block(t, lrange):
        NU = len(USTREAM)
        full = [(r, j, g) for r in range(HU + 1) for (j, g) in USTREAM]
        slots = []
        for pos, key in enumerate(full[E:E + HU * NU]):
            slots.append(('qk', key))
            if pos % 7 == 6:
                slots.append(('pv', divmod(pos // 7, NK)))
        sched = {}
        for c in range(HU * NK):
            for n in range(NL):
                sched[max(c * 8 + 2 * n, 1 + n if c == 0 else 0)] = (c, n)
        row64 = pl.multiple_of(t * 64, 64)
        row128 = pl.multiple_of(t * 128, 128)
        tn = (t + 1) % 4
        inx = jnp.minimum(i + (t + 1) // 4, NQ - 1)
        qbase = i * 4 + t
        qz, P, V, lsum, acc = {}, {}, {}, {}, {}
        lr = list(lrange)

        def get_qz(r):
            if r not in qz:
                qz[r] = qz_of(i, row64 + 8 * r, r) if r < HU else qz_of(inx, pl.multiple_of(tn * 64, 64), 0)
            return qz[r]

        def add_l(key, p):
            for a in (p[0:8], p[8:16]):
                lsum[key] = a if key not in lsum else lsum[key] + a

        def paced(a32, sl):
            if sl not in sched:
                return a32
            c, n = sched[sl]
            r, j = divmod(c, NK)
            zc = zs_ref[c * NL + n]
            kref = kb_scr.at[t + zc]
            qref = qf_scr.at[qbase + zc]

            def prod(d):
                return kref[d, j * 16:j * 16 + 16, :] * qref[pl.ds(d, 1), n * 128:(n + 1) * 128]

            sv = lax.fori_loop(r * DH + 1, (r + 1) * DH, lambda d, a: a + prod(d), prod(r * DH), unroll=True)
            p = jnp.exp2(sv)
            add_l((r, n), p)
            V[(c, n)] = p
            s32 = pltpu.bitcast(sv, u32)
            return a32 | ((s32[0:8] | s32[8:16]) & z_ref[...])

        def do_pv(r, j, sl):
            jt, jo = divmod(j * TK, TS)
            vt = pltpu.bitcast(paced(vt_scr[jt, pl.ds(row64 + 8 * r, 8), jo:jo + TK], sl), bf16)
            P[(r, j, 0)] = jnp.concatenate([V.pop((r * NK + j, n)) for n in range(NL)], axis=1)
            p = jnp.concatenate([P.pop((r, j, g)) for g in range(8)], axis=0).astype(bf16)
            a0 = acc[r] if r in acc else zacc[...]
            acc[r] = a0 + jnp.dot(vt, p, preferred_element_type=f32)
            if j == NK - 1:
                lt = lsum[r] + jnp.concatenate([lsum[(r, n)] for n in range(NL)], axis=1)
                l = jnp.sum(lt, axis=0, keepdims=True)
                inv = pl.reciprocal(l, approx=True)
                inv = inv * (2.0 - l * inv)
                ot_scr[pl.ds(row128 + DH * r, DH), :] = acc[r] * inv
                for n in range(NL):
                    lr[0] = jnp.minimum(lr[0], l[:, n * 128:(n + 1) * 128])
                    lr[1] = jnp.maximum(lr[1], l[:, n * 128:(n + 1) * 128])

        for n, key in enumerate(full[:E]):
            P[key] = pc_scr[n * 16:(n + 1) * 16, :]
            add_l(0, P[key])
        seg = []

        def flush():
            if not seg:
                return
            r = seg[0][0][0]
            kc = pltpu.bitcast(jnp.concatenate([kk for (_, kk) in seg], axis=0), bf16)
            pe = jnp.exp2(jnp.dot(kc, get_qz(r), preferred_element_type=f32))
            for n, (key, _) in enumerate(seg):
                p = pe[n * 16:(n + 1) * 16]
                if r < HU:
                    add_l(r, p)
                    P[key] = p
                else:
                    m = USTREAM.index(key[1:])
                    pc_scr[m * 16:(m + 1) * 16, :] = p
            seg.clear()

        for sl, (kind, key) in enumerate(slots):
            if kind == 'pv':
                flush()
                do_pv(key[0], key[1], sl)
            else:
                if seg and seg[0][0][0] != key[0]:
                    flush()
                r, j, g = key
                grp = j * 8 + g
                seg.append((key, paced(k_scr[t if r < HU else tn, grp * 8:(grp + 1) * 8, :], sl)))
        return tuple(lr)

    def safe_head(h, carry):
        slab = h // 8
        r = h % 8
        row8 = pl.multiple_of(h * 8, 8)
        qh = qt_scr[i, pl.ds(row8, 8), :]
        z = jnp.zeros_like(qh)
        qz = pltpu.bitcast(jnp.concatenate([jnp.where(r == n, qh, z) for n in range(8)], axis=0), bf16)

        def chunk(j, c):
            m, l, acc = c
            kc = pltpu.bitcast(k_scr[slab, pl.ds(pl.multiple_of(j * (TS // 2), TS // 2), TS // 2), :], bf16)
            s = jnp.dot(kc, qz, preferred_element_type=f32)
            mn = jnp.maximum(m, jnp.max(s, axis=0, keepdims=True))
            a = jnp.exp2(m - mn)
            p = jnp.exp2(s - mn)
            vt = pltpu.bitcast(vt_scr[j, pl.ds(row8, 8), :], bf16)
            l = l * a + jnp.sum(p, axis=0, keepdims=True)
            acc = acc * a + jnp.dot(vt, p.astype(bf16), preferred_element_type=f32)
            return mn, l, acc

        init = (jnp.full((1, TQ), -jnp.inf, f32), jnp.zeros((1, TQ), f32), jnp.zeros((DH, TQ), f32))
        _, l, acc = lax.fori_loop(0, S // TS, chunk, init)
        ot_scr[pl.ds(pl.multiple_of(h * DH, DH), DH), :] = acc / l
        return carry

    def out_cp(e):
        row = pl.multiple_of(i * TQ + e * HR, HR)
        return pltpu.make_async_copy(os_scr.at[e * HR:(e + 1) * HR], o_hbm.at[pl.ds(row, HR)], osems.at[e])

    def epilogue(c):
        attempt, _ = c

        @pl.when(attempt == 1)
        def _():
            lax.fori_loop(0, H, safe_head, 0)

        @pl.when(i + attempt > 0)
        def _():
            for e in range(EH):
                out_cp(e).wait()

        b1 = b1_scr[...].astype(f32).reshape(1, F)
        b2 = b2_scr[...].astype(f32).reshape(1, D)
        h1 = []
        for e in range(EH):
            o = ot_scr[:, e * HR:(e + 1) * HR].T.astype(bf16)
            xq = x_scr[i, e * (HR // TK):(e + 1) * (HR // TK)].reshape(HR, D).astype(f32)
            h1.append(xq + jnp.dot(o, wo_scr[...], preferred_element_type=f32))
        gs = []
        for e in range(EH):
            ln2 = _ln(h1[e]).astype(bf16)
            gs.append(_gelu(jnp.dot(ln2, w1_scr[...], preferred_element_type=f32) + b1).astype(bf16))
        ok = (lm_scr[0:1, :] >= L_LO) & (lm_scr[1:2, :] <= L_HI) & (vmax_scr[...] <= V_HI)
        nbad = jnp.max(jnp.where(ok, 0, 1))
        for e in range(EH):
            y = jnp.dot(gs[e], w2_scr[...], preferred_element_type=f32) + b2
            os_scr[e * HR:(e + 1) * HR, :] = (h1[e] + y).astype(bf16)
            out_cp(e).start()
        return attempt + 1, 1 + nbad

    pl.when(i == 0)(prologue)
    one = jnp.ones((1, 128), f32)
    lmin, lmax = lax.fori_loop(0, H // HU, block, (one, one))
    lm_scr[0:1, :] = lmin
    lm_scr[1:2, :] = lmax
    lax.while_loop(lambda c: c[0] < c[1], epilogue, (jnp.int32(0), jnp.int32(1)))

    @pl.when(i == NQ - 1)
    def _():
        for e in range(EH):
            out_cp(e).wait()


@jax.jit
def pallas_sequential_preLN__softmax_full_mha__dense_activation_gelu__prompt_kernel(
    A_x: jax.Array,
    A_wqkv: jax.Array,
    A_wo: jax.Array,
    B_x: jax.Array,
    B_w1: jax.Array,
    B_b1: jax.Array,
    B_w2: jax.Array,
    B_b2: jax.Array,
):
    del B_x
    hbm = pl.BlockSpec(memory_space=pl.ANY)
    out = pl.pallas_call(
        _kernel,
        grid=(NQ,),
        in_specs=[hbm] * 7,
        out_specs=hbm,
        out_shape=jax.ShapeDtypeStruct((S, D), bf16),
        scratch_shapes=[
            pltpu.VMEM((NQ, CPC, TK, D), bf16),
            pltpu.VMEM((NK, 16, D), bf16),
            pltpu.VMEM((D, D), bf16),
            pltpu.VMEM((D, D), bf16),
            pltpu.VMEM((D, D), bf16),
            pltpu.VMEM((D, D), bf16),
            pltpu.VMEM((D, F), bf16),
            pltpu.VMEM((F, D), bf16),
            pltpu.SemaphoreType.DMA((13,)),
            pltpu.VMEM((4, S // 2, 128), u32),
            pltpu.VMEM((4, 128, NK * 16, 128), f32),
            pltpu.VMEM((NQ, D // 2, TQ), u32),
            pltpu.VMEM((NQ * 4, 128, TQ), f32),
            pltpu.VMEM((S // TS, D // 2, TS), u32),
            pltpu.VMEM((D, TQ), f32),
            pltpu.VMEM((E * 16, TQ), f32),
            pltpu.VMEM((DH, TQ), f32),
            pltpu.VMEM((8, 128), u32),
            pltpu.SMEM((NZ,), jnp.int32),
            pltpu.VMEM((8, 128), f32),
            pltpu.VMEM((8, 128), f32),
            pltpu.VMEM((TQ, D), bf16),
            pltpu.SemaphoreType.DMA((EH,)),
            pltpu.VMEM((F,), bf16),
            pltpu.VMEM((D,), bf16),
        ],
        compiler_params=pltpu.CompilerParams(
            dimension_semantics=("arbitrary",), vmem_limit_bytes=120 * 1024 * 1024),
    )(A_x.reshape(NK, TK, D), A_wqkv, A_wo, B_w1, B_b1, B_w2, B_b2)
    return out.reshape(1, S, D)
```

```python
import math

import jax
import jax.numpy as jnp
from jax import lax
import jax.experimental.pallas as pl
import jax.experimental.pallas.tpu as pltpu

S, D, H, DH, F = 2048, 512, 32, 16, 1792
LOG2E = 1.4426950408889634
f32, bf16, u32 = jnp.float32, jnp.bfloat16, jnp.uint32

TQ = 512
TK = 128
NQ = S // TQ
NK = S // TK
NL = TQ // 128
HU = 8
CPC = TQ // TK
TS = 256
E = 10
EH = 4
HR = TQ // EH
NZ = HU * NK * NL
L_LO, L_HI, V_HI = 2.0 ** -20, 2.0 ** 90, 2.0 ** 30
NT = (((1,), (1,)), ((), ()))
USTREAM = [(j, g) for j in range(NK) for g in reversed(range(1, 8))]


def _ln(x):
    m = jnp.mean(x, axis=-1, keepdims=True)
    xc = x - m
    v = jnp.mean(xc * xc, axis=-1, keepdims=True)
    return xc * lax.rsqrt(v + 1e-5)


def _gelu(x):
    c = math.sqrt(2.0 / math.pi)
    return 0.5 * x * (1.0 + jnp.tanh(c * (x + 0.044715 * (x * x * x))))


def _pk(x):
    return [pltpu.bitcast(x[:, n * 128:(n + 1) * 128].astype(bf16), u32) for n in range(x.shape[1] // 128)]


def _kernel(x_hbm, wqkv_hbm, wo_hbm, w1_hbm, b1_hbm, w2_hbm, b2_hbm, o_hbm,
            x_scr, xv_scr, wq_scr, wk_scr, wv_scr, wo_scr, w1_scr, w2_scr, sems,
            k_scr, kb_scr, qt_scr, qf_scr, vt_scr, ot_scr, pc_scr, zacc, z_ref, zs_ref,
            vmax_scr, lm_scr, os_scr, osems, b1_scr, b2_scr):
    i = pl.program_id(0)

    def qz_of(ti, row, r):
        parts = []
        if r > 0:
            parts.append(jnp.zeros((8 * r, TQ), u32))
        parts.append(qt_scr[ti, pl.ds(row, 8), :])
        if r < 7:
            parts.append(jnp.zeros((8 * (7 - r), TQ), u32))
        return pltpu.bitcast(jnp.concatenate(parts, axis=0), bf16)

    def prologue():
        cp_xv = pltpu.make_async_copy(x_hbm.at[:, 0:16, :], xv_scr, sems.at[0])
        cp_wk = pltpu.make_async_copy(wqkv_hbm.at[:, D:2 * D], wk_scr, sems.at[1])
        cp_wq = pltpu.make_async_copy(wqkv_hbm.at[:, 0:D], wq_scr, sems.at[2])
        cp_wv = pltpu.make_async_copy(wqkv_hbm.at[:, 2 * D:3 * D], wv_scr, sems.at[3])
        cp_x = [pltpu.make_async_copy(x_hbm.at[c * CPC:(c + 1) * CPC], x_scr.at[c], sems.at[4 + c])
                for c in range(NQ)]
        cp_late = [pltpu.make_async_copy(wo_hbm, wo_scr, sems.at[8]),
                   pltpu.make_async_copy(w1_hbm, w1_scr, sems.at[9]),
                   pltpu.make_async_copy(b1_hbm, b1_scr, sems.at[10]),
                   pltpu.make_async_copy(w2_hbm, w2_scr, sems.at[11]),
                   pltpu.make_async_copy(b2_hbm, b2_scr, sems.at[12])]
        for cp in (cp_xv, cp_wk, cp_x[0], cp_wq, cp_x[1], cp_wv, cp_x[2], cp_x[3]):
            cp.start()
        zacc[...] = jnp.zeros_like(zacc)
        z_ref[...] = jnp.zeros_like(z_ref)

        def zero_zs(n, c):
            zs_ref[n] = 0
            return c

        lax.fori_loop(0, NZ, zero_zs, 0, unroll=True)

        cp_xv.wait()
        lnv = _ln(xv_scr[...].reshape(NK * 16, D).astype(f32)).astype(bf16)
        cp_wk.wait()
        wk = wk_scr[...]
        kv = _pk(jnp.dot(lnv, wk, preferred_element_type=f32))
        for s in range(4):
            for j in range(NK):
                k_scr[s, j * 64:j * 64 + 8, :] = kv[s][j * 8:(j + 1) * 8]
        work = iter([(c, s) for c in range(128) for s in range(4)])

        def kb_some(n):
            for _ in range(n):
                c, s = next(work)
                b = jnp.broadcast_to(kv[s][:, c:c + 1], (NK * 8, 128))
                kb_scr[s, c] = pltpu.bitcast(b, bf16).astype(f32)

        lnm, lnf, wT, vmax = {}, {}, {}, []

        def do_ln(c):
            m = _ln(jnp.concatenate([x_scr[c, jj, 16:TK, :] for jj in range(CPC)], axis=0).astype(f32)).astype(bf16)
            rows = []
            for jj in range(CPC):
                j = c * CPC + jj
                lnm[j] = m[jj * 112:(jj + 1) * 112]
                rows += [lnv[j * 16:(j + 1) * 16], lnm[j]]
            lnf[c] = jnp.concatenate(rows, axis=0)

        def do_k(j0, j1):
            lhs = jnp.concatenate([lnm[j] for j in range(j0, j1)], axis=0)
            k = _pk(jnp.dot(lhs, wk, preferred_element_type=f32))
            for s in range(4):
                for j in range(j0, j1):
                    k_scr[s, j * 64 + 8:(j + 1) * 64, :] = k[s][(j - j0) * 56:(j - j0 + 1) * 56]

        def do_q(c):
            qt = lax.dot_general(wT['q'], lnf[c], NT, preferred_element_type=f32) * (DH ** -0.5 * LOG2E)
            for n, pk in enumerate(_pk(qt)):
                qt_scr[c, :, n * 128:(n + 1) * 128] = pk
            for s in range(4):
                qf_scr[c * 4 + s] = qt[s * 128:(s + 1) * 128]

        def do_v(c):
            vtf = lax.dot_general(wT['v'], lnf[c], NT, preferred_element_type=f32)
            va = jnp.max(jnp.abs(vtf).reshape(D // 8, 8, TQ), axis=0)
            for n in range(NL):
                vn = va[:, n * 128:(n + 1) * 128]
                vmax[:] = [jnp.maximum(vmax[0], vn) if vmax else vn]
            for n, pk in enumerate(_pk(vtf)):
                jt, jo = divmod(c * TQ + n * 128, TS)
                vt_scr[jt, :, jo:jo + 128] = pk

        kb_some(8)
        cp_x[0].wait()
        do_ln(0)
        do_k(0, 2)
        kb_some(28)
        cp_wq.wait()
        cp_x[1].wait()
        wT['q'] = wq_scr[...].astype(f32).T.astype(bf16)
        do_ln(1)
        do_k(2, 4)
        kb_some(46)
        do_q(0)
        kb_some(46)
        do_k(4, 8)
        cp_wv.wait()
        cp_x[2].wait()
        cp_x[3].wait()
        for cp in cp_late:
            cp.start()
        wT['v'] = wv_scr[...].astype(f32).T.astype(bf16)
        rest = 512 - 8 - 28 - 92
        seq = [lambda: do_q(1), lambda: do_v(0), lambda: do_ln(2), lambda: do_v(1), lambda: do_k(8, 12),
               lambda: do_ln(3), lambda: do_q(2), lambda: do_v(2), lambda: do_k(12, 16), lambda: do_q(3),
               lambda: do_v(3)]
        done = 0
        for n, fn in enumerate(seq):
            fn()
            tgt = min(rest, (rest * (n + 1)) // (len(seq) - 1))
            kb_some(tgt - done)
            done = tgt
        kc = jnp.concatenate([k_scr[0, (j * 8 + g) * 8:(j * 8 + g) * 8 + 8, :] for (j, g) in USTREAM[:E]], axis=0)
        pc_scr[...] = jnp.exp2(jnp.dot(pltpu.bitcast(kc, bf16), qz_of(0, 0, 0), preferred_element_type=f32))
        vmax_scr[...] = vmax[0]
        for cp in cp_late:
            cp.wait()

    def block(t, lrange):
        NU = len(USTREAM)
        full = [(r, j, g) for r in range(HU + 1) for (j, g) in USTREAM]
        slots = []
        for pos, key in enumerate(full[E:E + HU * NU]):
            slots.append(('qk', key))
            if pos % 7 == 6:
                slots.append(('pv', divmod(pos // 7, NK)))
        sched = {}
        for c in range(HU * NK):
            for n in range(NL):
                sched[(3, 5, 6, 7)[n] if c == 0 else c * 8 + 2 * n + 1] = (c, n)
        row64 = pl.multiple_of(t * 64, 64)
        row128 = pl.multiple_of(t * 128, 128)
        tn = (t + 1) % 4
        inx = jnp.minimum(i + (t + 1) // 4, NQ - 1)
        qbase = i * 4 + t
        qz, P, V, lsum, acc = {}, {}, {}, {}, {}
        lr = list(lrange)

        def get_qz(r):
            if r not in qz:
                qz[r] = qz_of(i, row64 + 8 * r, r) if r < HU else qz_of(inx, pl.multiple_of(tn * 64, 64), 0)
            return qz[r]

        def flip_tiles(a):
            return jnp.concatenate([a[:, n * 128:(n + 1) * 128] for n in reversed(range(NL))], axis=1)

        def add_l(key, p):
            for a in (p[0:8], p[8:16]):
                lsum[key] = a if key not in lsum else lsum[key] + a

        def paced(a32, sl):
            if sl not in sched:
                return a32
            c, n = sched[sl]
            r, j = divmod(c, NK)
            zc = zs_ref[c * NL + n]
            kref = kb_scr.at[t + zc]
            qref = qf_scr.at[qbase + zc]

            def prod(d):
                return kref[d, j * 16:j * 16 + 16, :] * qref[pl.ds(d, 1), n * 128:(n + 1) * 128]

            sv = lax.fori_loop(r * DH + 1, (r + 1) * DH, lambda d, a: a + prod(d), prod(r * DH), unroll=True)
            p = jnp.exp2(sv)
            add_l((r, n), p)
            V[(c, n)] = p
            return a32 | (pltpu.bitcast(lsum[(r, n)], u32) & z_ref[...])

        def do_pv(r, j, sl):
            jt, jo = divmod(j * TK, TS)
            vt = pltpu.bitcast(paced(vt_scr[jt, pl.ds(row64 + 8 * r, 8), jo:jo + TK], sl), bf16)
            P[(r, j, 0)] = jnp.concatenate([V.pop((r * NK + j, n)) for n in range(NL)], axis=1)
            p = jnp.concatenate([P.pop((r, j, g)) for g in range(8)], axis=0)
            p = flip_tiles(p).astype(bf16)
            a0 = acc[r] if r in acc else zacc[...]
            acc[r] = a0 + jnp.dot(vt, p, preferred_element_type=f32)
            if j == NK - 1:
                lt = lsum[r] + jnp.concatenate([lsum[(r, n)] for n in range(NL)], axis=1)
                l = jnp.sum(lt, axis=0, keepdims=True)
                inv = pl.reciprocal(l, approx=True)
                inv = inv * (2.0 - l * inv)
                ot_scr[pl.ds(row128 + DH * r, DH), :] = flip_tiles(acc[r]) * inv
                for n in range(NL):
                    lr[0] = jnp.minimum(lr[0], l[:, n * 128:(n + 1) * 128])
                    lr[1] = jnp.maximum(lr[1], l[:, n * 128:(n + 1) * 128])

        for n, key in enumerate(full[:E]):
            P[key] = pc_scr[n * 16:(n + 1) * 16, :]
            add_l(0, P[key])
        seg = []

        def flush():
            if not seg:
                return
            r = seg[0][0][0]
            kc = pltpu.bitcast(jnp.concatenate([kk for (_, kk) in seg], axis=0), bf16)
            pe = jnp.exp2(jnp.dot(kc, get_qz(r), preferred_element_type=f32))
            for n, (key, _) in enumerate(seg):
                p = pe[n * 16:(n + 1) * 16]
                if r < HU:
                    add_l(r, p)
                    P[key] = p
                else:
                    m = USTREAM.index(key[1:])
                    pc_scr[m * 16:(m + 1) * 16, :] = p
            seg.clear()

        for sl, (kind, key) in enumerate(slots):
            if kind == 'pv':
                flush()
                do_pv(key[0], key[1], sl)
            else:
                if seg and seg[0][0][0] != key[0]:
                    flush()
                r, j, g = key
                grp = j * 8 + g
                seg.append((key, paced(k_scr[t if r < HU else tn, grp * 8:(grp + 1) * 8, :], sl)))
        return tuple(lr)

    def safe_head(h, carry):
        slab = h // 8
        r = h % 8
        row8 = pl.multiple_of(h * 8, 8)
        qh = qt_scr[i, pl.ds(row8, 8), :]
        z = jnp.zeros_like(qh)
        qz = pltpu.bitcast(jnp.concatenate([jnp.where(r == n, qh, z) for n in range(8)], axis=0), bf16)

        def chunk(j, c):
            m, l, acc = c
            kc = pltpu.bitcast(k_scr[slab, pl.ds(pl.multiple_of(j * (TS // 2), TS // 2), TS // 2), :], bf16)
            s = jnp.dot(kc, qz, preferred_element_type=f32)
            mn = jnp.maximum(m, jnp.max(s, axis=0, keepdims=True))
            a = jnp.exp2(m - mn)
            p = jnp.exp2(s - mn)
            vt = pltpu.bitcast(vt_scr[j, pl.ds(row8, 8), :], bf16)
            l = l * a + jnp.sum(p, axis=0, keepdims=True)
            acc = acc * a + jnp.dot(vt, p.astype(bf16), preferred_element_type=f32)
            return mn, l, acc

        init = (jnp.full((1, TQ), -jnp.inf, f32), jnp.zeros((1, TQ), f32), jnp.zeros((DH, TQ), f32))
        _, l, acc = lax.fori_loop(0, S // TS, chunk, init)
        ot_scr[pl.ds(pl.multiple_of(h * DH, DH), DH), :] = acc / l
        return carry

    def out_cp(e):
        row = pl.multiple_of(i * TQ + e * HR, HR)
        return pltpu.make_async_copy(os_scr.at[e * HR:(e + 1) * HR], o_hbm.at[pl.ds(row, HR)], osems.at[e])

    def epilogue(c):
        attempt, _ = c

        @pl.when(attempt == 1)
        def _():
            lax.fori_loop(0, H, safe_head, 0)

        @pl.when(i + attempt > 0)
        def _():
            for e in range(EH):
                out_cp(e).wait()

        b1 = b1_scr[...].astype(f32).reshape(1, F)
        b2 = b2_scr[...].astype(f32).reshape(1, D)
        h1 = []
        for e in range(EH):
            o = ot_scr[:, e * HR:(e + 1) * HR].T.astype(bf16)
            xq = x_scr[i, e * (HR // TK):(e + 1) * (HR // TK)].reshape(HR, D).astype(f32)
            h1.append(xq + jnp.dot(o, wo_scr[...], preferred_element_type=f32))
        gs = []
        for e in range(EH):
            ln2 = _ln(h1[e]).astype(bf16)
            gs.append(_gelu(jnp.dot(ln2, w1_scr[...], preferred_element_type=f32) + b1).astype(bf16))
        ok = (lm_scr[0:1, :] >= L_LO) & (lm_scr[1:2, :] <= L_HI) & (vmax_scr[...] <= V_HI)
        nbad = jnp.max(jnp.where(ok, 0, 1))
        for e in range(EH):
            y = jnp.dot(gs[e], w2_scr[...], preferred_element_type=f32) + b2
            os_scr[e * HR:(e + 1) * HR, :] = (h1[e] + y).astype(bf16)
            out_cp(e).start()
        return attempt + 1, 1 + nbad

    pl.when(i == 0)(prologue)
    one = jnp.ones((1, 128), f32)
    lmin, lmax = lax.fori_loop(0, H // HU, block, (one, one))
    lm_scr[0:1, :] = lmin
    lm_scr[1:2, :] = lmax
    lax.while_loop(lambda c: c[0] < c[1], epilogue, (jnp.int32(0), jnp.int32(1)))

    @pl.when(i == NQ - 1)
    def _():
        for e in range(EH):
            out_cp(e).wait()


@jax.jit
def pallas_sequential_preLN__softmax_full_mha__dense_activation_gelu__prompt_kernel(
    A_x: jax.Array,
    A_wqkv: jax.Array,
    A_wo: jax.Array,
    B_x: jax.Array,
    B_w1: jax.Array,
    B_b1: jax.Array,
    B_w2: jax.Array,
    B_b2: jax.Array,
):
    del B_x
    hbm = pl.BlockSpec(memory_space=pl.ANY)
    out = pl.pallas_call(
        _kernel,
        grid=(NQ,),
        in_specs=[hbm] * 7,
        out_specs=hbm,
        out_shape=jax.ShapeDtypeStruct((S, D), bf16),
        scratch_shapes=[
            pltpu.VMEM((NQ, CPC, TK, D), bf16),
            pltpu.VMEM((NK, 16, D), bf16),
            pltpu.VMEM((D, D), bf16),
            pltpu.VMEM((D, D), bf16),
            pltpu.VMEM((D, D), bf16),
            pltpu.VMEM((D, D), bf16),
            pltpu.VMEM((D, F), bf16),
            pltpu.VMEM((F, D), bf16),
            pltpu.SemaphoreType.DMA((13,)),
            pltpu.VMEM((4, S // 2, 128), u32),
            pltpu.VMEM((4, 128, NK * 16, 128), f32),
            pltpu.VMEM((NQ, D // 2, TQ), u32),
            pltpu.VMEM((NQ * 4, 128, TQ), f32),
            pltpu.VMEM((S // TS, D // 2, TS), u32),
            pltpu.VMEM((D, TQ), f32),
            pltpu.VMEM((E * 16, TQ), f32),
            pltpu.VMEM((DH, TQ), f32),
            pltpu.VMEM((8, 128), u32),
            pltpu.SMEM((NZ,), jnp.int32),
            pltpu.VMEM((8, 128), f32),
            pltpu.VMEM((8, 128), f32),
            pltpu.VMEM((TQ, D), bf16),
            pltpu.SemaphoreType.DMA((EH,)),
            pltpu.VMEM((F,), bf16),
            pltpu.VMEM((D,), bf16),
        ],
        compiler_params=pltpu.CompilerParams(
            dimension_semantics=("arbitrary",), vmem_limit_bytes=120 * 1024 * 1024),
    )(A_x.reshape(NK, TK, D), A_wqkv, A_wo, B_w1, B_b1, B_w2, B_b2)
    return out.reshape(1, S, D)
```

```python
import math

import jax
import jax.numpy as jnp
from jax import lax
import jax.experimental.pallas as pl
import jax.experimental.pallas.tpu as pltpu

S, D, H, DH, F = 2048, 512, 32, 16, 1792
LOG2E = 1.4426950408889634
f32, bf16, u32 = jnp.float32, jnp.bfloat16, jnp.uint32

TQ = 512
TK = 128
NQ = S // TQ
NK = S // TK
NL = TQ // 128
HU = 8
CPC = TQ // TK
TS = 256
E = 10
EH = 4
HR = TQ // EH
NZ = HU * NK * NL
L_LO, L_HI, V_HI = 2.0 ** -20, 2.0 ** 90, 2.0 ** 30
NT = (((1,), (1,)), ((), ()))
USTREAM = [(j, g) for j in range(NK) for g in reversed(range(1, 8))]


def _ln(x):
    m = jnp.mean(x, axis=-1, keepdims=True)
    xc = x - m
    v = jnp.mean(xc * xc, axis=-1, keepdims=True)
    return xc * lax.rsqrt(v + 1e-5)


def _gelu(x):
    c = math.sqrt(2.0 / math.pi)
    return 0.5 * x * (1.0 + jnp.tanh(c * (x + 0.044715 * (x * x * x))))


def _pk(x):
    return [pltpu.bitcast(x[:, n * 128:(n + 1) * 128].astype(bf16), u32) for n in range(x.shape[1] // 128)]


def _kernel(x_hbm, wqkv_hbm, wo_hbm, w1_hbm, b1_hbm, w2_hbm, b2_hbm, o_hbm,
            x_scr, xv_scr, wq_scr, wk_scr, wv_scr, wo_scr, w1_scr, w2_scr, sems,
            k_scr, kb_scr, qt_scr, qf_scr, vt_scr, ot_scr, pc_scr, zacc, z_ref, zs_ref,
            vmax_scr, lm_scr, os_scr, osems, b1_scr, b2_scr):
    i = pl.program_id(0)

    def qz_of(ti, row, r):
        parts = []
        if r > 0:
            parts.append(jnp.zeros((8 * r, TQ), u32))
        parts.append(qt_scr[ti, pl.ds(row, 8), :])
        if r < 7:
            parts.append(jnp.zeros((8 * (7 - r), TQ), u32))
        return pltpu.bitcast(jnp.concatenate(parts, axis=0), bf16)

    def prologue():
        cp_xv = pltpu.make_async_copy(x_hbm.at[:, 0:16, :], xv_scr, sems.at[0])
        cp_wk = pltpu.make_async_copy(wqkv_hbm.at[:, D:2 * D], wk_scr, sems.at[1])
        cp_wq = pltpu.make_async_copy(wqkv_hbm.at[:, 0:D], wq_scr, sems.at[2])
        cp_wv = pltpu.make_async_copy(wqkv_hbm.at[:, 2 * D:3 * D], wv_scr, sems.at[3])
        cp_x = [pltpu.make_async_copy(x_hbm.at[c * CPC:(c + 1) * CPC], x_scr.at[c], sems.at[4 + c])
                for c in range(NQ)]
        cp_late = [pltpu.make_async_copy(wo_hbm, wo_scr, sems.at[8]),
                   pltpu.make_async_copy(w1_hbm, w1_scr, sems.at[9]),
                   pltpu.make_async_copy(b1_hbm, b1_scr, sems.at[10]),
                   pltpu.make_async_copy(w2_hbm, w2_scr, sems.at[11]),
                   pltpu.make_async_copy(b2_hbm, b2_scr, sems.at[12])]
        for cp in (cp_xv, cp_wk, cp_x[0], cp_wq, cp_x[1], cp_wv, cp_x[2], cp_x[3]):
            cp.start()
        zacc[...] = jnp.zeros_like(zacc)
        z_ref[...] = jnp.zeros_like(z_ref)

        def zero_zs(n, c):
            zs_ref[n] = 0
            return c

        lax.fori_loop(0, NZ, zero_zs, 0, unroll=True)

        cp_xv.wait()
        lnv = _ln(xv_scr[...].reshape(NK * 16, D).astype(f32)).astype(bf16)
        cp_wk.wait()
        wk = wk_scr[...]
        kv = _pk(jnp.dot(lnv, wk, preferred_element_type=f32))
        for s in range(4):
            for j in range(NK):
                k_scr[s, j * 64:j * 64 + 8, :] = kv[s][j * 8:(j + 1) * 8]
        work = iter([(c, s) for c in range(128) for s in range(4)])

        def kb_some(n):
            for _ in range(n):
                c, s = next(work)
                b = jnp.broadcast_to(kv[s][:, c:c + 1], (NK * 8, 128))
                kb_scr[s, c] = pltpu.bitcast(b, bf16).astype(f32)

        lnm, lnf, wT, vmax = {}, {}, {}, []

        def do_ln(c):
            m = _ln(jnp.concatenate([x_scr[c, jj, 16:TK, :] for jj in range(CPC)], axis=0).astype(f32)).astype(bf16)
            rows = []
            for jj in range(CPC):
                j = c * CPC + jj
                lnm[j] = m[jj * 112:(jj + 1) * 112]
                rows += [lnv[j * 16:(j + 1) * 16], lnm[j]]
            lnf[c] = jnp.concatenate(rows, axis=0)

        def do_k(j0, j1):
            lhs = jnp.concatenate([lnm[j] for j in range(j0, j1)], axis=0)
            k = _pk(jnp.dot(lhs, wk, preferred_element_type=f32))
            for s in range(4):
                for j in range(j0, j1):
                    k_scr[s, j * 64 + 8:(j + 1) * 64, :] = k[s][(j - j0) * 56:(j - j0 + 1) * 56]

        def do_q(c):
            qt = lax.dot_general(wT['q'], lnf[c], NT, preferred_element_type=f32) * (DH ** -0.5 * LOG2E)
            for n, pk in enumerate(_pk(qt)):
                qt_scr[c, :, n * 128:(n + 1) * 128] = pk
            for s in range(4):
                qf_scr[c * 4 + s] = qt[s * 128:(s + 1) * 128]

        def do_v(c):
            vtf = lax.dot_general(wT['v'], lnf[c], NT, preferred_element_type=f32)
            va = jnp.max(jnp.abs(vtf).reshape(D // 8, 8, TQ), axis=0)
            for n in range(NL):
                vn = va[:, n * 128:(n + 1) * 128]
                vmax[:] = [jnp.maximum(vmax[0], vn) if vmax else vn]
            for n, pk in enumerate(_pk(vtf)):
                jt, jo = divmod(c * TQ + n * 128, TS)
                vt_scr[jt, :, jo:jo + 128] = pk

        kb_some(8)
        cp_x[0].wait()
        do_ln(0)
        do_k(0, 2)
        kb_some(28)
        cp_wq.wait()
        cp_x[1].wait()
        wT['q'] = wq_scr[...].astype(f32).T.astype(bf16)
        do_ln(1)
        do_k(2, 4)
        kb_some(46)
        do_q(0)
        kb_some(46)
        do_k(4, 8)
        cp_wv.wait()
        cp_x[2].wait()
        cp_x[3].wait()
        for cp in cp_late:
            cp.start()
        wT['v'] = wv_scr[...].astype(f32).T.astype(bf16)
        rest = 512 - 8 - 28 - 92
        seq = [lambda: do_q(1), lambda: do_v(0), lambda: do_ln(2), lambda: do_v(1), lambda: do_k(8, 12),
               lambda: do_ln(3), lambda: do_q(2), lambda: do_v(2), lambda: do_k(12, 16), lambda: do_q(3),
               lambda: do_v(3)]
        done = 0
        for n, fn in enumerate(seq):
            fn()
            tgt = min(rest, (rest * (n + 1)) // (len(seq) - 1))
            kb_some(tgt - done)
            done = tgt
        kc = jnp.concatenate([k_scr[0, (j * 8 + g) * 8:(j * 8 + g) * 8 + 8, :] for (j, g) in USTREAM[:E]], axis=0)
        pc_scr[...] = jnp.exp2(jnp.dot(pltpu.bitcast(kc, bf16), qz_of(0, 0, 0), preferred_element_type=f32))
        vmax_scr[...] = vmax[0]
        for cp in cp_late:
            cp.wait()

    def block(t, lrange):
        NU = len(USTREAM)
        full = [(r, j, g) for r in range(HU + 1) for (j, g) in USTREAM]
        slots = []
        for pos, key in enumerate(full[E:E + HU * NU]):
            slots.append(('qk', key))
            if pos % 7 == 6:
                slots.append(('pv', divmod(pos // 7, NK)))
        sched = {}
        for c in range(HU * NK):
            for n in range(NL):
                sched[(3, 5, 6, 7)[n] if c == 0 else c * 8 + 2 * n + 1] = (c, n)
        row64 = pl.multiple_of(t * 64, 64)
        row128 = pl.multiple_of(t * 128, 128)
        tn = (t + 1) % 4
        inx = jnp.minimum(i + (t + 1) // 4, NQ - 1)
        qbase = i * 4 + t
        qz, P, V, lsum, acc = {}, {}, {}, {}, {}
        lr = list(lrange)

        def get_qz(r):
            if r not in qz:
                qz[r] = qz_of(i, row64 + 8 * r, r) if r < HU else qz_of(inx, pl.multiple_of(tn * 64, 64), 0)
            return qz[r]

        def flip_tiles(a):
            return jnp.concatenate([a[:, n * 128:(n + 1) * 128] for n in reversed(range(NL))], axis=1)

        def add_l(key, p):
            for a in (p[0:8], p[8:16]):
                lsum[key] = a if key not in lsum else lsum[key] + a

        def paced(a32, sl):
            if sl not in sched:
                return a32
            c, n = sched[sl]
            r, j = divmod(c, NK)
            zc = zs_ref[c * NL + n]
            kref = kb_scr.at[t + zc]
            qref = qf_scr.at[qbase + zc]

            def prod(d):
                return kref[d, j * 16:j * 16 + 16, :] * qref[pl.ds(d, 1), n * 128:(n + 1) * 128]

            sv = lax.fori_loop(r * DH + 1, (r + 1) * DH, lambda d, a: a + prod(d), prod(r * DH), unroll=True)
            p = jnp.exp2(sv)
            add_l((r, n), p)
            V[(c, n)] = p
            return a32 | (pltpu.bitcast(lsum[(r, n)], u32) & z_ref[...])

        def do_pv(r, j, sl):
            jt, jo = divmod(j * TK, TS)
            vt = pltpu.bitcast(paced(vt_scr[jt, pl.ds(row64 + 8 * r, 8), jo:jo + TK], sl), bf16)
            P[(r, j, 0)] = jnp.concatenate([V.pop((r * NK + j, n)) for n in range(NL)], axis=1)
            p = jnp.concatenate([P.pop((r, j, g)) for g in range(8)], axis=0)
            p = flip_tiles(p).astype(bf16)
            a0 = acc[r] if r in acc else zacc[...]
            acc[r] = a0 + jnp.dot(vt, p, preferred_element_type=f32)
            if j == NK - 1:
                lt = lsum[r] + jnp.concatenate([lsum[(r, n)] for n in range(NL)], axis=1)
                l = jnp.sum(lt, axis=0, keepdims=True)
                inv = pl.reciprocal(l, approx=True)
                inv = inv * (2.0 - l * inv)
                ot_scr[pl.ds(row128 + DH * r, DH), :] = flip_tiles(acc[r]) * inv
                for n in range(NL):
                    lr[0] = jnp.minimum(lr[0], l[:, n * 128:(n + 1) * 128])
                    lr[1] = jnp.maximum(lr[1], l[:, n * 128:(n + 1) * 128])

        for n, key in enumerate(full[:E]):
            P[key] = pc_scr[n * 16:(n + 1) * 16, :]
            add_l(0, P[key])
        seg = []

        def flush():
            if not seg:
                return
            r = seg[0][0][0]
            kc = pltpu.bitcast(jnp.concatenate([kk for (_, kk) in seg], axis=0), bf16)
            pe = jnp.exp2(jnp.dot(kc, get_qz(r), preferred_element_type=f32))
            for n, (key, _) in enumerate(seg):
                p = pe[n * 16:(n + 1) * 16]
                if r < HU:
                    add_l(r, p)
                    P[key] = p
                else:
                    m = USTREAM.index(key[1:])
                    pc_scr[m * 16:(m + 1) * 16, :] = p
            seg.clear()

        for sl, (kind, key) in enumerate(slots):
            if kind == 'pv':
                flush()
                do_pv(key[0], key[1], sl)
            else:
                if seg and seg[0][0][0] != key[0]:
                    flush()
                r, j, g = key
                grp = j * 8 + g
                seg.append((key, paced(k_scr[t if r < HU else tn, grp * 8:(grp + 1) * 8, :], sl)))
        return tuple(lr)

    def safe_head(h, carry):
        slab = h // 8
        r = h % 8
        row8 = pl.multiple_of(h * 8, 8)
        qh = qt_scr[i, pl.ds(row8, 8), :]
        z = jnp.zeros_like(qh)
        qz = pltpu.bitcast(jnp.concatenate([jnp.where(r == n, qh, z) for n in range(8)], axis=0), bf16)

        def chunk(j, c):
            m, l, acc = c
            kc = pltpu.bitcast(k_scr[slab, pl.ds(pl.multiple_of(j * (TS // 2), TS // 2), TS // 2), :], bf16)
            s = jnp.dot(kc, qz, preferred_element_type=f32)
            mn = jnp.maximum(m, jnp.max(s, axis=0, keepdims=True))
            a = jnp.exp2(m - mn)
            p = jnp.exp2(s - mn)
            vt = pltpu.bitcast(vt_scr[j, pl.ds(row8, 8), :], bf16)
            l = l * a + jnp.sum(p, axis=0, keepdims=True)
            acc = acc * a + jnp.dot(vt, p.astype(bf16), preferred_element_type=f32)
            return mn, l, acc

        init = (jnp.full((1, TQ), -jnp.inf, f32), jnp.zeros((1, TQ), f32), jnp.zeros((DH, TQ), f32))
        _, l, acc = lax.fori_loop(0, S // TS, chunk, init)
        ot_scr[pl.ds(pl.multiple_of(h * DH, DH), DH), :] = acc / l
        return carry

    def out_cp(e, tile):
        row = pl.multiple_of(tile * TQ + e * HR, HR)
        return pltpu.make_async_copy(os_scr.at[e * HR:(e + 1) * HR], o_hbm.at[pl.ds(row, HR)], osems.at[e])

    def epilogue(c):
        attempt, _ = c

        @pl.when(attempt == 1)
        def _():
            lax.fori_loop(0, H, safe_head, 0)

        @pl.when(i + attempt > 0)
        def _():
            for e in range(EH):
                out_cp(e, i - 1 + attempt).wait()

        b1 = b1_scr[...].astype(f32).reshape(1, F)
        b2 = b2_scr[...].astype(f32).reshape(1, D)
        h1 = []
        for e in range(EH):
            o = ot_scr[:, e * HR:(e + 1) * HR].T.astype(bf16)
            xq = x_scr[i, e * (HR // TK):(e + 1) * (HR // TK)].reshape(HR, D).astype(f32)
            h1.append(xq + jnp.dot(o, wo_scr[...], preferred_element_type=f32))
        gs = []
        for e in range(EH):
            ln2 = _ln(h1[e]).astype(bf16)
            gs.append(_gelu(jnp.dot(ln2, w1_scr[...], preferred_element_type=f32) + b1).astype(bf16))
        ok = (lm_scr[0:1, :] >= L_LO) & (lm_scr[1:2, :] <= L_HI) & (vmax_scr[...] <= V_HI)
        nbad = jnp.max(jnp.where(ok, 0, 1))
        for e in range(EH):
            y = jnp.dot(gs[e], w2_scr[...], preferred_element_type=f32) + b2
            os_scr[e * HR:(e + 1) * HR, :] = (h1[e] + y).astype(bf16)
            out_cp(e, i).start()
        return attempt + 1, 1 + nbad

    pl.when(i == 0)(prologue)
    one = jnp.ones((1, 128), f32)
    lmin, lmax = lax.fori_loop(0, H // HU, block, (one, one))
    lm_scr[0:1, :] = lmin
    lm_scr[1:2, :] = lmax
    lax.while_loop(lambda c: c[0] < c[1], epilogue, (jnp.int32(0), jnp.int32(1)))

    @pl.when(i == NQ - 1)
    def _():
        for e in range(EH):
            out_cp(e, i).wait()


@jax.jit
def pallas_sequential_preLN__softmax_full_mha__dense_activation_gelu__prompt_kernel(
    A_x: jax.Array,
    A_wqkv: jax.Array,
    A_wo: jax.Array,
    B_x: jax.Array,
    B_w1: jax.Array,
    B_b1: jax.Array,
    B_w2: jax.Array,
    B_b2: jax.Array,
):
    del B_x
    hbm = pl.BlockSpec(memory_space=pl.ANY)
    out = pl.pallas_call(
        _kernel,
        grid=(NQ,),
        in_specs=[hbm] * 7,
        out_specs=hbm,
        out_shape=jax.ShapeDtypeStruct((S, D), bf16),
        scratch_shapes=[
            pltpu.VMEM((NQ, CPC, TK, D), bf16),
            pltpu.VMEM((NK, 16, D), bf16),
            pltpu.VMEM((D, D), bf16),
            pltpu.VMEM((D, D), bf16),
            pltpu.VMEM((D, D), bf16),
            pltpu.VMEM((D, D), bf16),
            pltpu.VMEM((D, F), bf16),
            pltpu.VMEM((F, D), bf16),
            pltpu.SemaphoreType.DMA((13,)),
            pltpu.VMEM((4, S // 2, 128), u32),
            pltpu.VMEM((4, 128, NK * 16, 128), f32),
            pltpu.VMEM((NQ, D // 2, TQ), u32),
            pltpu.VMEM((NQ * 4, 128, TQ), f32),
            pltpu.VMEM((S // TS, D // 2, TS), u32),
            pltpu.VMEM((D, TQ), f32),
            pltpu.VMEM((E * 16, TQ), f32),
            pltpu.VMEM((DH, TQ), f32),
            pltpu.VMEM((8, 128), u32),
            pltpu.SMEM((NZ,), jnp.int32),
            pltpu.VMEM((8, 128), f32),
            pltpu.VMEM((8, 128), f32),
            pltpu.VMEM((TQ, D), bf16),
            pltpu.SemaphoreType.DMA((EH,)),
            pltpu.VMEM((F,), bf16),
            pltpu.VMEM((D,), bf16),
        ],
        compiler_params=pltpu.CompilerParams(
            dimension_semantics=("arbitrary",), vmem_limit_bytes=120 * 1024 * 1024),
    )(A_x.reshape(NK, TK, D), A_wqkv, A_wo, B_w1, B_b1, B_w2, B_b2)
    return out.reshape(1, S, D)
```
